```python
import jax
import jax.numpy as jnp

def _softmax(x, axis=-1):
    return jax.nn.softmax(x, axis=axis)
def _gelu(x):
    return jax.nn.gelu(x, approximate=True)
def _silu(x):
    return jax.nn.silu(x)
def _sigmoid(x):
    return jax.nn.sigmoid(x)
def _layernorm(x, axis=-1, eps=1e-5):
    m = jnp.mean(x, axis=axis, keepdims=True)
    v = jnp.var(x, axis=axis, keepdims=True)
    return (x - m) / jnp.sqrt(v + eps)
def _scatter_add(tgt, idx, src, axis=0):
    return tgt.at[idx].add(src)
def _segment_sum(src, seg, n):
    return jax.ops.segment_sum(src, seg, n)
class _Rng:
    def __init__(self, key):
        self._k = key
    def _next(self):
        self._k, sub = jax.random.split(self._k)
        return sub
    def normal(self, shape):
        return jax.random.normal(self._next(), shape, dtype=jnp.bfloat16)
    def randint(self, lo, hi, shape):
        return jax.random.randint(self._next(), shape, lo, hi, dtype=jnp.int32)
    def uniform(self, shape, lo=0.0, hi=1.0):
        return jax.random.uniform(self._next(), shape, jnp.bfloat16, lo, hi)
    def permutation(self, n):
        return jax.random.permutation(self._next(), n)


kernel_name = 'standalone__structured_sparse_n_m__ragged'

def setup_inputs():
    _rng = _Rng(jax.random.key(int.from_bytes(__import__("os").urandom(4), "little")))
    _w = (lambda a: (lambda t: t.astype(jnp.bfloat16) if jnp.issubdtype(t.dtype, jnp.floating) else t)(jnp.asarray(a)))
    B, S, D = 16, 4096, 576
    assert D % 4 == 0, "d_model must be divisible by M=4 for 2:4 sparsity"
    return {
        "x": _w((lambda *s: _rng.normal(s) * 0.05)(B, S, D)),
        "w": _w((lambda *s: _rng.normal(s) * 0.05)(D, D)),
        "b": _w((lambda *s: _rng.normal(s) * 0.05)(D)),
    }

def reference(x, w, b):
    B, S, D = x.shape
    N, M = 2, 4
    G = D // M
    wg = w.reshape(G, M, D)
    mag = jnp.abs(wg)
    order = jnp.argsort(mag, 1)
    thr = jnp.take_along_axis(mag, order[:, M - N:M - N + 1, :], 1)
    mask = (lambda x, dt: x.astype(dt))(mag >= thr, w.dtype)
    wp = (wg * mask).reshape(D, D)
    return jnp.einsum("bsd,df->bsf", x, wp) + b
```

```python
import jax
import jax.numpy as jnp
from jax import lax
import jax.experimental.pallas as pl
import jax.experimental.pallas.tpu as pltpu

F32, BF16 = jnp.float32, jnp.bfloat16
KB = 64
PIECE = 256
RING = 9
FIRST = 4
W_FROM = 124

S1, S2, S4, S3, S0 = (0, 2), (1, 3), (4, 6), (5, 7), (8,)


def _product(s, a, b):
    n = len(s)
    return ({(i, s[k]): a[n * i + k] for i in range(2) for k in range(n) if a[n * i + k]},
            {(s[k], j): b[2 * k + j] for k in range(n) for j in range(2) if b[2 * k + j]})


PASSES = dict(
    AB=(_product(S1, (1, 0, -1, 0), (-1, 1, 0, 0)), _product(S2, (1, 0, -.5, 0), (-2, 1, 0, 0))),
    BA=(_product(S1, (0, 1, 0, -1), (0, 0, -1, 1)), _product(S2, (0, 1, 0, -.5), (0, 0, -2, 1))),
    G1=(_product(S1, (0, 1, -1, 0), (1, 0, 0, 1)), _product(S2, (0, 1, -.5, 0), (2, 0, 0, 1))),
    AA=(_product(S4, (-.5, 0, 1, 0), (-2, 1, 0, 0)), _product(S3, (-1, 0, 1, 0), (-1, 1, 0, 0))),
    BB=(_product(S4, (0, -.5, 0, 1), (0, 0, -2, 1)), _product(S3, (0, -1, 0, 1), (0, 0, -1, 1))),
    G2=(_product(S4, (0, -.5, 1, 0), (0, 1, 2, 0)), _product(S3, (0, -1, 1, 0), (0, 1, 1, 0))),
    AC=(_product(S1, (1, -1, 0, 0), (1, 0, 0, 0)), _product(S3, (1, -1, 0, 0), (0, 1, 0, 0))),
    BC=(_product(S1, (0, 0, -1, 1), (0, 0, 0, 1)), _product(S3, (0, 0, -1, 1), (0, 0, 1, 0))),
    CA=(_product(S1, (0, 1, 0, 0), (1, 0, 1, 0)), _product(S3, (0, 0, 1, 0), (1, 0, 1, 0))),
    CB=(_product(S1, (0, 0, 1, 0), (0, 1, 0, 1)), _product(S3, (0, 1, 0, 0), (0, 1, 0, 1))),
    AD=(_product(S4, (.5, -.5, 0, 0), (0, 1, 0, 0)), _product(S2, (1, -1, 0, 0), (1, 0, 0, 0))),
    BD=(_product(S4, (0, 0, -1, 1), (0, 0, 1, 0)), _product(S2, (0, 0, -.5, .5), (0, 0, 0, 1))),
    DA=(_product(S0, (-1 / 3, 2 / 3), (1, 0)), _product(S2, (0, 1, 0, 0), (1, 0, 1, 0))),
    DB=(_product(S0, (-1 / 3, 2 / 3), (0, 1)), _product(S2, (0, 0, .5, 0), (0, 1, 0, 1))),
    EA=(_product(S4, (0, 0, 1, 0), (1, 0, 1, 0)), _product(S0, (2 / 3, -1 / 3), (1, 0))),
    EB=(_product(S4, (0, .5, 0, 0), (0, 1, 0, 1)), _product(S0, (2 / 3, -1 / 3), (0, 1))),
)
SLOT = {name: i for i, name in enumerate(PASSES)}


def _prune_packed(u):
    mate = lax.broadcasted_iota(jnp.int32, u.shape, 0) ^ 1
    lo = pltpu.bitcast((u << 16) & 0x7FFFFFFF, F32)
    hi = pltpu.bitcast(u & 0x7FFF0000, F32)
    big, small = jnp.maximum(lo, hi), jnp.minimum(lo, hi)
    nbig = jnp.take_along_axis(big, mate, axis=0, mode="promise_in_bounds")
    nsmall = jnp.take_along_axis(small, mate, axis=0, mode="promise_in_bounds")
    thr = jnp.maximum(jnp.minimum(big, nbig), jnp.maximum(small, nsmall))
    return u & (jnp.where(lo < thr, 0, 0xFFFF) | jnp.where(hi < thr, 0, -65536))


def _combine(terms):
    acc = None
    for c, v in sorted(terms, key=lambda t: t[0] < 0):
        if acc is None:
            acc = v if c == 1 else c * v
        else:
            v = v if abs(c) == 1 else abs(c) * v
            acc = acc + v if c > 0 else acc - v
    return acc


def _kernel(x_hbm, w_hbm, b_hbm, o_hbm, xbuf, obuf, wbuf, bbuf, wc_ref, bias_ref,
            xsem, fsem, wsem, osem):
    NB, D, S = x_hbm.shape
    F = w_hbm.shape[1]
    H = F // 2
    per = S // PIECE

    def read(b, slot):
        return pltpu.make_async_copy(x_hbm.at[b], xbuf.at[slot], xsem.at[slot])

    def read_first(j):
        n = FIRST * PIECE
        cols = pl.ds(pl.multiple_of(j * n, n), n)
        return pltpu.make_async_copy(x_hbm.at[0, :, cols], xbuf.at[0, :, cols], fsem.at[j])

    def write(p):
        cols = pl.ds(pl.multiple_of((p & (per - 1)) * PIECE, PIECE), PIECE)
        return pltpu.make_async_copy(
            obuf.at[p], o_hbm.at[p >> (per.bit_length() - 1), :, cols], osem.at[0])

    wcp = pltpu.make_async_copy(w_hbm, wbuf, wsem.at[0])
    bcp = pltpu.make_async_copy(b_hbm, bbuf, wsem.at[1])
    wcp.start()
    bcp.start()
    for j in range(per // FIRST):
        read_first(j).start(priority=1)
    for b in range(1, RING):
        read(b, b).start(priority=1)
    wcp.wait()
    bcp.wait()
    u = pltpu.bitcast(wbuf[...], jnp.int32)
    parts = [_prune_packed(u[8 * i:8 * i + 8]) for i in range(D // 16)]
    parts += parts[-KB // 16:]
    wt = pltpu.bitcast(jnp.concatenate(parts, axis=0), BF16).T.astype(F32)
    low = lax.broadcasted_iota(jnp.int32, (H, 128), 1) < KB
    for name, halves in PASSES.items():
        lo, hi = (_combine([(c, wt[i * H:(i + 1) * H, k // 2 * 128:(k // 2 + 1) * 128])
                            for (i, k), c in wform.items()]) for wform, _ in halves)
        wc_ref[SLOT[name]] = pltpu.bitcast(jnp.where(low, lo, hi).astype(BF16), jnp.int32)
    bias_ref[...] = jnp.broadcast_to(bbuf[...].reshape(1, F).astype(F32), (128, F)).T

    def piece(slot, col, p):
        def block(k, j):
            return pltpu.bitcast(xbuf[slot, pl.ds(k * KB, KB), pl.ds(col + j * 128, 128)], jnp.uint32)

        def operand(xform):
            if len(xform) == 1:
                return block(*next(iter(xform)))
            return pltpu.pack_elementwise(
                [_combine([(c, pltpu.unpack_elementwise(
                    block(k, j), index=h, packed_dtype=BF16, unpacked_dtype=F32))
                    for (k, j), c in xform.items()]) for h in range(2)], packed_dtype=BF16)

        def mm(name):
            rhs = jnp.concatenate([operand(xform) for _, xform in PASSES[name]], axis=0)
            return jnp.dot(pltpu.bitcast(wc_ref[SLOT[name]], BF16), pltpu.bitcast(rhs, BF16),
                           preferred_element_type=F32)

        def put(i, j, v):
            obuf[p, pl.ds(i * H, H), pl.ds(j * 128, 128)] = v.astype(obuf.dtype)

        AC, AD, G1, G2 = mm("AC"), mm("AD"), mm("G1"), mm("G2")
        s = AC + AD + bias_ref[0:H]
        c11 = s - G2
        c12 = s + AD + G1
        BC, BD, BA, BB = mm("BC"), mm("BD"), mm("BA"), mm("BB")
        s = BC + BD + bias_ref[H:F]
        c21 = s + BA - G1
        c22 = s + BD + BB + G2
        CA, DA, EA, AA = mm("CA"), mm("DA"), mm("EA"), mm("AA")
        s = CA + DA + EA
        put(0, 0, s + EA + AA + c11)
        put(1, 0, s + DA + c21)
        CB, DB, EB, AB = mm("CB"), mm("DB"), mm("EB"), mm("AB")
        s = CB + DB + EB
        put(0, 1, s + EB + AB + c12)
        put(1, 1, s + DB + c22)

    def first_batch(j, carry):
        read_first(j).wait()
        for i in range(FIRST):
            p = j * FIRST + i
            piece(0, pl.multiple_of(p * PIECE, PIECE), p)
        return carry

    lax.fori_loop(0, per // FIRST, first_batch, 0)
    read(RING, 0).start(priority=1)

    def batch(t, slot):
        read(t, slot).wait()
        for i in range(per):
            p = t * per + i
            piece(slot, i * PIECE, p)
            done = jnp.minimum(2 * (p - W_FROM), p)
            upto = jnp.minimum(2 * (p - W_FROM) + 2, p + 1)
            for q in range(2):
                @pl.when(jnp.logical_and(p >= W_FROM, done + q < upto))
                def _():
                    write(done + q).start()

        @pl.when(t + RING < NB)
        def _():
            read(t + RING, slot).start(priority=1)
        return jnp.where(slot == RING - 1, 0, slot + 1)

    lax.fori_loop(1, NB, batch, 1)
    pltpu.make_async_copy(obuf, obuf, osem.at[0]).wait()


@jax.jit
def pallas_standalone__structured_sparse_n_m__ragged_kernel(
    x: jax.Array,
    w: jax.Array,
    b: jax.Array,
):
    B, S, D = x.shape
    F = w.shape[1]
    assert D == 9 * KB and S // PIECE <= W_FROM <= B * S // PIECE // 2
    xt = jnp.transpose(x, (0, 2, 1))
    out = pl.pallas_call(
        _kernel,
        in_specs=[pl.BlockSpec(memory_space=pl.ANY)] * 3,
        out_specs=pl.BlockSpec(memory_space=pl.ANY),
        out_shape=jax.ShapeDtypeStruct((B, F, S), x.dtype),
        scratch_shapes=[
            pltpu.VMEM((RING, D, S), x.dtype),
            pltpu.VMEM((B * S // PIECE, F, PIECE), x.dtype),
            pltpu.VMEM((D, F), w.dtype),
            pltpu.VMEM((F,), b.dtype),
            pltpu.VMEM((len(PASSES), F // 4, 128), jnp.int32),
            pltpu.VMEM((F, 128), F32),
            pltpu.SemaphoreType.DMA((RING,)),
            pltpu.SemaphoreType.DMA((S // PIECE // FIRST,)),
            pltpu.SemaphoreType.DMA((2,)),
            pltpu.SemaphoreType.DMA((1,)),
        ],
        compiler_params=pltpu.CompilerParams(
            vmem_limit_bytes=127 * 1024 * 1024,
            disable_bounds_checks=True,
            disable_semaphore_checks=True,
        ),
    )(xt, w, b)
    return jnp.transpose(out, (0, 2, 1))
```

```python
import jax
import jax.numpy as jnp
from jax import lax
import jax.experimental.pallas as pl
import jax.experimental.pallas.tpu as pltpu

F32, BF16, U32 = jnp.float32, jnp.bfloat16, jnp.uint32

STRASSEN = {
    1: ({(0, 0): 1, (1, 1): 1}, {(0, 0): 1, (1, 1): 1}),
    2: ({(1, 0): 1, (1, 1): 1}, {(0, 0): 1}),
    3: ({(0, 0): 1}, {(0, 1): 1, (1, 1): -1}),
    4: ({(1, 1): 1}, {(1, 0): 1, (0, 0): -1}),
    5: ({(0, 0): 1, (0, 1): 1}, {(1, 1): 1}),
    6: ({(1, 0): 1, (0, 0): -1}, {(0, 0): 1, (0, 1): 1}),
    7: ({(0, 1): 1, (1, 1): -1}, {(1, 0): 1, (1, 1): 1}),
}
RESULT = {(0, 0): {1: 1, 4: 1, 5: -1, 7: 1}, (0, 1): {3: 1, 5: 1},
          (1, 0): {2: 1, 4: 1}, (1, 1): {1: 1, 2: -1, 3: 1, 6: 1}}
NESTED = (2, 3, 4, 5)
ORDER = (None, (1, 4), (0, 2), (0, 1), None, (1, 2), (0, 4), (1, 1),
         (0, 5), (0, 7), (1, 5), (1, 7), (1, 3), (0, 3), (1, 6), (0, 6))
GROUP_WORK = 16 + 2 * (7 * 8 - len(NESTED))

RING = 18
LEAD = 2
W_FROM = 244
READ_ORDER = tuple(8 * i + r for r in range(8) for i in range(9))


def _combine(terms):
    terms = list(terms)
    acc = terms.pop(next(k for k, (c, _) in enumerate(terms) if c > 0))[1]
    for c, v in terms:
        acc = acc + v if c > 0 else acc - v
    return acc


def _pack_rows(v):
    n = v.shape[0] // 16
    v = v.reshape(n, 2, 8, v.shape[1])
    return pltpu.pack_elementwise([v[:, h].reshape(8 * n, -1) for h in range(2)], packed_dtype=BF16)


def _prune_packed(u):
    mate = lax.broadcasted_iota(jnp.int32, u.shape, 0) ^ 1
    lo = pltpu.bitcast((u << 16) & 0x7FFFFFFF, F32)
    hi = pltpu.bitcast(u & 0x7FFF0000, F32)
    big, small = jnp.maximum(lo, hi), jnp.minimum(lo, hi)
    nbig = jnp.take_along_axis(big, mate, axis=0, mode="promise_in_bounds")
    nsmall = jnp.take_along_axis(small, mate, axis=0, mode="promise_in_bounds")
    thr = jnp.maximum(jnp.minimum(big, nbig), jnp.maximum(small, nsmall))
    return u & (jnp.where(lo < thr, 0, 0xFFFF) | jnp.where(hi < thr, 0, -65536))


def _weight_forms():
    tall, short = {}, {}
    for g in range(2):
        tile = lambda k, s: 2 * k + s if 2 * k + s < 3 else 3 + g
        for m, (a, _) in STRASSEN.items():
            if m in NESTED:
                for n, (a2, _) in STRASSEN.items():
                    short[g, m, n] = tuple(sorted(
                        ((2 * i + i2, tile(k, s)), c * c2)
                        for (i, k), c in a.items() for (i2, s), c2 in a2.items()))
            else:
                for s in range(2):
                    tall[g, m, s] = tuple(sorted(((2 * i, tile(k, s)), c) for (i, k), c in a.items()))
    for q in range(4):
        short["E", q] = (((q, 5), 1),)
    return tall, short


def _distinct(forms):
    return list(dict.fromkeys(forms.values()))


def _prepare_weights(wbuf, tall_ref, short_ref):
    D, F = wbuf.shape
    u = pltpu.bitcast(wbuf[...], jnp.int32)
    rows = [_pack_rows(pltpu.bitcast(_prune_packed(u[8 * i:8 * i + 8]), BF16).astype(F32))
            for i in range(D // 16)]
    rows = rows[:32] + rows[24:28] + rows[32:36] + rows[28:36]
    a = pltpu.bitcast(pltpu.bitcast(jnp.concatenate(rows, axis=0), BF16).T, U32)
    where = {}
    for forms, ref in zip(_weight_forms(), (tall_ref, short_ref)):
        n = ref.shape[1]
        block = lambda q, t: a[q * F // 8:q * F // 8 + n, t * 128:(t + 1) * 128]
        for slot, form in enumerate(_distinct(forms)):
            if len(form) == 1:
                ref[slot] = block(*form[0][0])
            else:
                ref[slot] = pltpu.pack_elementwise([_combine(
                    (c, pltpu.unpack_elementwise(block(q, t), index=h, packed_dtype=BF16, unpacked_dtype=F32))
                    for (q, t), c in form) for h in range(2)], packed_dtype=BF16)
        where.update({name: (ref, _distinct(forms).index(form)) for name, form in forms.items()})
    return lambda *name: pltpu.bitcast(where[name][0][where[name][1]], BF16)


def _group(load, weights, bias_ref, store, progress):
    Q = bias_ref.shape[0] // 4
    loaded, prods, shared, stored, arrival = {}, {}, {}, set(), []

    def x_blocks(k, n, pair, h):
        if (k, n, pair) not in loaded:
            words = load(k, n, pair).reshape(64 * n, 128)
            loaded[k, n, pair] = pltpu.bitcast(words, BF16).astype(F32).reshape(8 * n, 2, 8, 128)
        return loaded[k, n, pair][:, h].reshape(64 * n, 128)

    def x_tile(g, t, j, h):
        if t < 3:
            return x_blocks(2 * t, 2, 2 * g + j, h)
        diff = x_blocks(7 + g, 1, 2 * g + j, h) - x_blocks(7 + g, 1, 2 * (1 - g) + j, h)
        return jnp.concatenate([x_blocks(6, 1, 2 * g + j, h), diff], axis=0)

    def dot(a, b):
        return jnp.dot(a, pltpu.bitcast(_pack_rows(b), BF16), preferred_element_type=F32)

    e_todo = [(2 * i + q, j, h) for i, j in ((1, 0), (0, 0), (0, 1), (1, 1))
              for h in range(2) for q in range(2)]

    def shared_pass():
        q, j, h = e_todo.pop(0)
        rhs = jnp.concatenate([x_blocks(7, 1, 2 + j, h), x_blocks(8, 1, j, h)], axis=0)
        shared[q, j, h] = dot(weights("E", q), rhs) + bias_ref[pl.ds(q * Q, Q)]
        arrival.append(("E", q // 2, j))
        progress(1)

    def product(g, m):
        operand = lambda s, h: _combine(
            (c, x_tile(g, 2 * k + s, j, h)) for (k, j), c in STRASSEN[m][1].items())
        if m in NESTED:
            mm = lambda n: dot(weights(g, m, n), _combine(
                (c, operand(s, h)) for (s, h), c in STRASSEN[n][1].items()))
            n5, n1, n4, n7 = mm(5), mm(1), mm(4), mm(7)
            c11 = (n1 + n4) + (n7 - n5)
            progress(4)
            n2, n3, n6 = mm(2), mm(3), mm(6)
            shared_pass()
            progress(3)
            prods[g, m] = (jnp.concatenate([c11, n2 + n4], axis=0),
                           jnp.concatenate([n3 + n5, n6 + (n3 - n2) + n1], axis=0))
        else:
            p = [dot(weights(g, m, s), operand(s, h)) for h in range(2) for s in range(2)]
            prods[g, m] = (p[0] + p[1], p[2] + p[3])
            progress(8)
        arrival.append((g, m))

    def finish(g, i, j):
        values = []
        for h in range(2):
            terms = {(g, m): (c, prods[g, m][h]) for m, c in RESULT[i, j].items()}
            terms["E", i, j] = (1, jnp.concatenate([shared[2 * i + q, j, h] for q in range(2)], axis=0))
            values.append(_combine(terms[k] for k in sorted(terms, key=arrival[::-1].index)))
        store(i, 2 * g + j, values)

    for step in ORDER:
        if step is None:
            for _ in range(4):
                shared_pass()
        else:
            product(*step)
        loaded.clear()
        for g in range(2):
            for (i, j), ms in RESULT.items():
                if ((g, i, j) not in stored and all((g, m) in prods for m in ms)
                        and (2 * i + 1, j, 1) in shared):
                    finish(g, i, j)
                    stored.add((g, i, j))
    assert len(stored) == 8


def _kernel(x_hbm, w_hbm, b_hbm, o_hbm, xbuf, obuf, wbuf, bbuf, tall_ref, short_ref, bias_ref,
            xsem, wsem, osem):
    F = w_hbm.shape[1]
    NC = obuf.shape[0]
    x_words = x_hbm.bitcast(U32)

    def read(c, slot, i, r, priority):
        pltpu.make_async_copy(x_words.at[c >> 1, i, r, pl.ds((c & 1) * 8, 8)],
                              xbuf.at[slot, i, r], xsem.at[slot]).start(priority=priority)

    def write(c, r, q):
        pltpu.make_async_copy(obuf.at[c, :, r, pl.ds(2 * q, 2)],
                              o_hbm.at[c >> 1, :, r, pl.ds((c & 1) * 8 + 2 * q, 2)], osem.at[0]).start()

    def write_eighth(n):
        for q in range(4):
            write(n >> 3, 2 * (n & 3) + ((n >> 2) & 1), q)

    params = [pltpu.make_async_copy(w_hbm, wbuf, wsem.at[0]),
              pltpu.make_async_copy(b_hbm, bbuf, wsem.at[1])]
    for copy in params:
        copy.start()
    for c in range(LEAD):
        for r in range(8):
            read(c, c, slice(None), r, 1)
    for copy in params:
        copy.wait()
    weights = _prepare_weights(wbuf, tall_ref, short_ref)
    bias_ref[...] = jnp.broadcast_to(bbuf[...].reshape(1, F).astype(F32), (128, F)).T

    wrap = lambda s: jnp.where(s >= RING, s - RING, s)

    def chunk(t, carry):
        slot, next_slot, written = carry
        pltpu.make_async_copy(xbuf.at[slot], xbuf.at[slot], xsem.at[slot]).wait()
        next_slots = (next_slot, wrap(next_slot + 1))
        work = 0

        def progress(n):
            nonlocal work, written
            before, work = work, work + n
            per = len(READ_ORDER)
            due = range(before * per // GROUP_WORK, work * per // GROUP_WORK)
            for h in range(2):
                ks = [k - h * per for k in due if k // per == h]
                if ks:
                    @pl.when(LEAD + 2 * t + h < NC)
                    def _():
                        for k in ks:
                            read(LEAD + 2 * t + h, next_slots[h], *divmod(READ_ORDER[k], 8), k % 2)
            for k in range(pl.cdiv(before * 8, GROUP_WORK), pl.cdiv(work * 8, GROUP_WORK)):
                go = jnp.logical_and(16 * t + k >= W_FROM, written < 8 * t)
                pl.when(go)(lambda: write_eighth(written))
                written = written + go.astype(jnp.int32)
            if before < GROUP_WORK * 6 // 5 <= work:
                @pl.when(t == NC - 1)
                def _():
                    for r in range(8):
                        for q in range(2):
                            write(t, r, q)

        for u in range(2):
            def load(k, n, pair):
                return xbuf[slot, pl.ds(k, n), :, 4 * u + pair]

            def store(i, pair, values):
                v = jnp.concatenate([a.reshape(36, 8, 128) for a in values], axis=1).astype(obuf.dtype)
                whole, part = (v[:32], v[32:]) if i == 0 else (v[4:], v[:4])
                obuf[t, pl.ds(5 * i, 4), :, 4 * u + pair] = whole.reshape(4, 8, 16, 128)
                obuf[t, 4, pl.ds(4 * i, 4), 4 * u + pair] = part

            _group(load, weights, bias_ref, store, progress)
        return wrap(slot + 1), wrap(next_slot + 2), written

    _, _, written = lax.fori_loop(0, NC, chunk, (0, LEAD, 0))
    lax.fori_loop(written, 8 * (NC - 1), lambda n, _: write_eighth(n), None)
    for r in range(8):
        for q in range(2, 4):
            write(NC - 1, r, q)
    pltpu.make_async_copy(obuf, obuf, osem.at[0]).wait()


@jax.jit
def pallas_standalone__structured_sparse_n_m__ragged_kernel(
    x: jax.Array,
    w: jax.Array,
    b: jax.Array,
):
    B, S, D = x.shape
    F = w.shape[1]
    assert (S, D, F) == (4096, 576, 576) and B < RING
    tall, short = _weight_forms()
    xt = jnp.transpose(x.reshape(B, 32, 128, 9, 8, 8), (0, 3, 4, 1, 5, 2)).reshape(B, 9, 8, 16, 16, 128)
    out = pl.pallas_call(
        _kernel,
        in_specs=[pl.BlockSpec(memory_space=pl.ANY)] * 3,
        out_specs=pl.BlockSpec(memory_space=pl.ANY),
        out_shape=jax.ShapeDtypeStruct(xt.shape, x.dtype),
        scratch_shapes=[
            pltpu.VMEM((RING, 9, 8, 8, 8, 128), U32),
            pltpu.VMEM((2 * B, 9, 8, 8, 16, 128), x.dtype),
            pltpu.VMEM((D, F), w.dtype),
            pltpu.VMEM((F,), b.dtype),
            pltpu.VMEM((len(_distinct(tall)), F // 4, 128), U32),
            pltpu.VMEM((len(_distinct(short)), F // 8, 128), U32),
            pltpu.VMEM((F, 128), F32),
            pltpu.SemaphoreType.DMA((RING,)),
            pltpu.SemaphoreType.DMA((2,)),
            pltpu.SemaphoreType.DMA((1,)),
        ],
        compiler_params=pltpu.CompilerParams(
            vmem_limit_bytes=128 * 1024 * 1024,
            disable_bounds_checks=True,
            disable_semaphore_checks=True,
        ),
    )(xt, w, b)
    return jnp.transpose(out.reshape(B, 9, 8, 32, 8, 128), (0, 3, 5, 1, 2, 4)).reshape(B, S, F)
```

```python
import jax
import jax.numpy as jnp
from jax import lax
import jax.experimental.pallas as pl
import jax.experimental.pallas.tpu as pltpu

F32, BF16, U32 = jnp.float32, jnp.bfloat16, jnp.uint32

STRASSEN = {
    1: ({(0, 0): 1, (1, 1): 1}, {(0, 0): 1, (1, 1): 1}),
    2: ({(1, 0): 1, (1, 1): 1}, {(0, 0): 1}),
    3: ({(0, 0): 1}, {(0, 1): 1, (1, 1): -1}),
    4: ({(1, 1): 1}, {(1, 0): 1, (0, 0): -1}),
    5: ({(0, 0): 1, (0, 1): 1}, {(1, 1): 1}),
    6: ({(1, 0): 1, (0, 0): -1}, {(0, 0): 1, (0, 1): 1}),
    7: ({(0, 1): 1, (1, 1): -1}, {(1, 0): 1, (1, 1): 1}),
}
RESULT = {(0, 0): {1: 1, 4: 1, 5: -1, 7: 1}, (0, 1): {3: 1, 5: 1},
          (1, 0): {2: 1, 4: 1}, (1, 1): {1: 1, 2: -1, 3: 1, 6: 1}}
NESTED = (2, 3, 4, 5)
ORDER = (None, (1, 4), (0, 2), (0, 1), None, (1, 2), (0, 4), (1, 1),
         (0, 5), (0, 7), (1, 5), (1, 7), (1, 3), (0, 3), (1, 6), (0, 6))
GROUP_WORK = 16 + 2 * (7 * 8 - len(NESTED))

RING = 9
DELAY = 34
W_FROM = 246
W_PHASE = 10
WIDE = 6
READ_ORDER = tuple(24 * i + -j % 24 for j in range(24) for i in range(6))


def _combine(terms):
    terms = list(terms)
    acc = terms.pop(next(k for k, (c, _) in enumerate(terms) if c > 0))[1]
    for c, v in terms:
        acc = acc + v if c > 0 else acc - v
    return acc


def _pack_rows(v):
    n = v.shape[0] // 16
    v = v.reshape(n, 2, 8, v.shape[1])
    return pltpu.pack_elementwise([v[:, h].reshape(8 * n, -1) for h in range(2)], packed_dtype=BF16)


def _prune_packed(u):
    mate = lax.broadcasted_iota(jnp.int32, u.shape, 0) ^ 1
    lo = pltpu.bitcast((u << 16) & 0x7FFFFFFF, F32)
    hi = pltpu.bitcast(u & 0x7FFF0000, F32)
    big, small = jnp.maximum(lo, hi), jnp.minimum(lo, hi)
    nbig = jnp.take_along_axis(big, mate, axis=0, mode="promise_in_bounds")
    nsmall = jnp.take_along_axis(small, mate, axis=0, mode="promise_in_bounds")
    thr = jnp.maximum(jnp.minimum(big, nbig), jnp.maximum(small, nsmall))
    return u & (jnp.where(lo < thr, 0, 0xFFFF) | jnp.where(hi < thr, 0, -65536))


def _weight_forms():
    tall, short = {}, {}
    for g in range(2):
        tile = lambda k, s: 2 * k + s if 2 * k + s < 3 else 3 + g
        for m, (a, _) in STRASSEN.items():
            if m in NESTED:
                for n, (a2, _) in STRASSEN.items():
                    short[g, m, n] = tuple(sorted(
                        ((2 * i + i2, tile(k, s)), c * c2)
                        for (i, k), c in a.items() for (i2, s), c2 in a2.items()))
            else:
                for s in range(2):
                    tall[g, m, s] = tuple(sorted(((2 * i, tile(k, s)), c) for (i, k), c in a.items()))
    for q in range(4):
        short["E", q] = (((q, 5), 1),)
    return tall, short


def _distinct(forms):
    return list(dict.fromkeys(forms.values()))


def _prepare_weights(wbuf, tall_ref, short_ref):
    D, F = wbuf.shape
    u = pltpu.bitcast(wbuf[...], jnp.int32)
    rows = [_pack_rows(pltpu.bitcast(_prune_packed(u[8 * i:8 * i + 8]), BF16).astype(F32))
            for i in range(D // 16)]
    rows = rows[:32] + rows[24:28] + rows[32:36] + rows[28:36]
    a = pltpu.bitcast(pltpu.bitcast(jnp.concatenate(rows, axis=0), BF16).T, U32)
    where = {}
    for forms, ref in zip(_weight_forms(), (tall_ref, short_ref)):
        n = ref.shape[1]
        block = lambda q, t: a[q * F // 8:q * F // 8 + n, t * 128:(t + 1) * 128]
        for slot, form in enumerate(_distinct(forms)):
            if len(form) == 1:
                ref[slot] = block(*form[0][0])
            else:
                ref[slot] = pltpu.pack_elementwise([_combine(
                    (c, pltpu.unpack_elementwise(block(q, t), index=h, packed_dtype=BF16, unpacked_dtype=F32))
                    for (q, t), c in form) for h in range(2)], packed_dtype=BF16)
        where.update({name: (ref, _distinct(forms).index(form)) for name, form in forms.items()})
    return lambda *name: pltpu.bitcast(where[name][0][where[name][1]], BF16)


def _group(load, weights, bias_ref, store, progress):
    Q = bias_ref.shape[0] // 4
    loaded, prods, shared, stored, arrival = {}, {}, {}, set(), []

    def x_blocks(k, n, pair, h):
        if (k, n, pair) not in loaded:
            words = load(k, n, pair).reshape(64 * n, 128)
            loaded[k, n, pair] = pltpu.bitcast(words, BF16).astype(F32).reshape(8 * n, 2, 8, 128)
        return loaded[k, n, pair][:, h].reshape(64 * n, 128)

    def x_tile(g, t, j, h):
        if t < 3:
            return x_blocks(2 * t, 2, 2 * g + j, h)
        diff = x_blocks(7 + g, 1, 2 * g + j, h) - x_blocks(7 + g, 1, 2 * (1 - g) + j, h)
        return jnp.concatenate([x_blocks(6, 1, 2 * g + j, h), diff], axis=0)

    def dot(a, b):
        return jnp.dot(a, pltpu.bitcast(_pack_rows(b), BF16), preferred_element_type=F32)

    e_todo = [(2 * i + q, j, h) for i, j in ((1, 0), (0, 0), (0, 1), (1, 1))
              for h in range(2) for q in range(2)]

    def shared_pass():
        q, j, h = e_todo.pop(0)
        rhs = jnp.concatenate([x_blocks(7, 1, 2 + j, h), x_blocks(8, 1, j, h)], axis=0)
        shared[q, j, h] = dot(weights("E", q), rhs) + bias_ref[pl.ds(q * Q, Q)]
        arrival.append(("E", q // 2, j))
        progress(1)

    def product(g, m):
        operand = lambda s, h: _combine(
            (c, x_tile(g, 2 * k + s, j, h)) for (k, j), c in STRASSEN[m][1].items())
        if m in NESTED:
            mm = lambda n: dot(weights(g, m, n), _combine(
                (c, operand(s, h)) for (s, h), c in STRASSEN[n][1].items()))
            n5, n1, n4, n7 = mm(5), mm(1), mm(4), mm(7)
            c11 = (n1 + n4) + (n7 - n5)
            progress(4)
            n2, n3, n6 = mm(2), mm(3), mm(6)
            shared_pass()
            progress(3)
            prods[g, m] = (jnp.concatenate([c11, n2 + n4], axis=0),
                           jnp.concatenate([n3 + n5, n6 + (n3 - n2) + n1], axis=0))
        else:
            p = [dot(weights(g, m, s), operand(s, h)) for h in range(2) for s in range(2)]
            prods[g, m] = (p[0] + p[1], p[2] + p[3])
            progress(8)
        arrival.append((g, m))

    def finish(g, i, j):
        values = []
        for h in range(2):
            terms = {(g, m): (c, prods[g, m][h]) for m, c in RESULT[i, j].items()}
            terms["E", i, j] = (1, jnp.concatenate([shared[2 * i + q, j, h] for q in range(2)], axis=0))
            values.append(_combine(terms[k] for k in sorted(terms, key=arrival[::-1].index)))
        store(i, 2 * g + j, values)

    for step in ORDER:
        if step is None:
            for _ in range(4):
                shared_pass()
        else:
            product(*step)
        loaded.clear()
        for g in range(2):
            for (i, j), ms in RESULT.items():
                if ((g, i, j) not in stored and all((g, m) in prods for m in ms)
                        and (2 * i + 1, j, 1) in shared):
                    finish(g, i, j)
                    stored.add((g, i, j))
    assert len(stored) == 8


def _kernel(x_hbm, w_hbm, b_hbm, o_hbm, xbuf, obuf, wbuf, bbuf, tall_ref, short_ref, bias_ref,
            xsem, first_sem, wsem, osem):
    F = w_hbm.shape[1]
    B = obuf.shape[0]
    x_words = x_hbm.bitcast(U32)
    o_wide, obuf_wide = (r.reshape(B // 2, 9, 16, 16, 16, 128) for r in (o_hbm, obuf))

    def read_first(u):
        for r in range(8):
            at = (0, slice(None), r, pl.ds(4 * u, 4))
            pltpu.make_async_copy(x_words.at[at], xbuf.at[at], first_sem.at[min(u, 2)]).start(priority=1)

    def read(b, slot, k):
        g = READ_ORDER[k]
        at = (g >> 4, (g >> 1) & 7, pl.ds(8 * (g & 1), 8))
        pltpu.make_async_copy(x_words.at[(b, *at)], xbuf.at[(slot, *at)], xsem.at[slot]).start(priority=k % 2)

    def arrived(groups, sem):
        part = xbuf.at[0, :, :, pl.ds(0, 4 * groups)]
        pltpu.make_async_copy(part, part, sem).wait()

    def write(b, r, q):
        at = (b, slice(None), r, pl.ds(2 * q, 2))
        pltpu.make_async_copy(obuf.at[at], o_hbm.at[at], osem.at[0]).start()

    def write_wide(n):
        for q in range(2):
            at = (n >> 5, slice(None), (n >> 1) & 15, pl.ds(8 * (n & 1) + 4 * q, 4))
            pltpu.make_async_copy(obuf_wide.at[at], o_wide.at[at], osem.at[0]).start()

    def write_narrow(n):
        for q in range(4):
            write(n >> 4, 2 * (n & 3) + ((n >> 2) & 1), ((n >> 1) & 4) + q)

    def write_group(u):
        for r in range(8):
            for q in range(2):
                write(B - 1, r, 2 * u + q)

    params = [pltpu.make_async_copy(b_hbm, bbuf, wsem.at[0]),
              pltpu.make_async_copy(w_hbm, wbuf, wsem.at[1])]
    for copy in params:
        copy.start()
    read_first(0)
    read_first(1)
    for copy in params:
        copy.wait()
    read_first(2)
    read_first(3)
    weights = _prepare_weights(wbuf, tall_ref, short_ref)
    bias_ref[...] = jnp.broadcast_to(bbuf[...].reshape(1, F).astype(F32), (128, F)).T

    wrap = lambda s: jnp.where(s >= RING, s - RING, s)

    def half_batch(t, carry):
        slot, read_slot, written = carry
        pl.when(t == 0)(lambda: arrived(1, first_sem.at[0]))
        pl.when(t == 1)(lambda: arrived(2, first_sem.at[2]))
        pl.when(jnp.logical_and(t > 1, t & 1 == 0))(lambda: arrived(4, xsem.at[slot]))
        read_slots = (read_slot, wrap(read_slot + 1))
        work = 0

        def progress(n):
            nonlocal work, written
            before, work = work, work + n
            per = len(READ_ORDER)
            due = range(*(per - DELAY + v * per // (2 * GROUP_WORK) for v in (before, work)))
            for h in range(2):
                ks = [k - h * per for k in due if k // per == h]
                if ks:
                    @pl.when(jnp.logical_and(t + h > 0, t + h < B))
                    def _():
                        for k in ks:
                            read(t + h, read_slots[h], k)
            for k in range(*(pl.cdiv((v - W_PHASE) * 8, GROUP_WORK) for v in (before, work))):
                wide = written < 32 * WIDE
                ready = jnp.where(wide, written | 31, written) < 8 * t
                go = jnp.logical_and(16 * t + k >= W_FROM, ready)
                pl.when(jnp.logical_and(go, wide))(lambda: write_wide(written))
                pl.when(jnp.logical_and(go, jnp.logical_not(wide)))(lambda: write_narrow(written))
                written = written + go.astype(jnp.int32)
            if before < GROUP_WORK * 6 // 5 <= work:
                pl.when(t == 2 * B - 1)(lambda: write_group(2))

        for u in range(2):
            first = (t & 1) * 8 + 4 * u

            def load(k, n, pair):
                return xbuf[slot, pl.ds(k, n), :, first + pair]

            def store(i, pair, values):
                v = jnp.concatenate([a.reshape(36, 8, 128) for a in values], axis=1).astype(obuf.dtype)
                whole, part = (v[:32], v[32:]) if i == 0 else (v[4:], v[:4])
                obuf[t >> 1, pl.ds(5 * i, 4), :, first + pair] = whole.reshape(4, 8, 16, 128)
                obuf[t >> 1, 4, pl.ds(4 * i, 4), first + pair] = part

            if u:
                pl.when(t == 0)(lambda: arrived(1, first_sem.at[1]))
            _group(load, weights, bias_ref, store, progress)
        return wrap(slot + (t & 1)), read_slots[1], written

    _, _, written = lax.fori_loop(0, 2 * B, half_batch, (0, 0, 0))
    lax.fori_loop(written, 8 * (2 * B - 1), lambda n, _: write_narrow(n), None)
    write_group(3)
    pltpu.make_async_copy(obuf, obuf, osem.at[0]).wait()


@jax.jit
def pallas_standalone__structured_sparse_n_m__ragged_kernel(
    x: jax.Array,
    w: jax.Array,
    b: jax.Array,
):
    B, S, D = x.shape
    F = w.shape[1]
    assert (B, S, D, F) == (16, 4096, 576, 576)
    tall, short = _weight_forms()
    xt = jnp.transpose(x.reshape(B, 32, 128, 9, 8, 8), (0, 3, 4, 1, 5, 2)).reshape(B, 9, 8, 16, 16, 128)
    out = pl.pallas_call(
        _kernel,
        in_specs=[pl.BlockSpec(memory_space=pl.ANY)] * 3,
        out_specs=pl.BlockSpec(memory_space=pl.ANY),
        out_shape=jax.ShapeDtypeStruct(xt.shape, x.dtype),
        scratch_shapes=[
            pltpu.VMEM((RING, 9, 8, 16, 8, 128), U32),
            pltpu.VMEM(xt.shape, x.dtype),
            pltpu.VMEM((D, F), w.dtype),
            pltpu.VMEM((F,), b.dtype),
            pltpu.VMEM((len(_distinct(tall)), F // 4, 128), U32),
            pltpu.VMEM((len(_distinct(short)), F // 8, 128), U32),
            pltpu.VMEM((F, 128), F32),
            pltpu.SemaphoreType.DMA((RING,)),
            pltpu.SemaphoreType.DMA((3,)),
            pltpu.SemaphoreType.DMA((2,)),
            pltpu.SemaphoreType.DMA((1,)),
        ],
        compiler_params=pltpu.CompilerParams(
            vmem_limit_bytes=128 * 1024 * 1024,
            disable_bounds_checks=True,
            disable_semaphore_checks=True,
            flags={"XLA_TPU_RESCHEDULE_DMA_DONES": True},
        ),
    )(xt, w, b)
    return jnp.transpose(out.reshape(B, 9, 8, 32, 8, 128), (0, 3, 5, 1, 2, 4)).reshape(B, S, F)
```

```python
import jax
import jax.numpy as jnp
from jax import lax
import jax.experimental.pallas as pl
import jax.experimental.pallas.tpu as pltpu

F32, BF16, U32 = jnp.float32, jnp.bfloat16, jnp.uint32

STRASSEN = {
    1: ({(0, 0): 1, (1, 1): 1}, {(0, 0): 1, (1, 1): 1}),
    2: ({(1, 0): 1, (1, 1): 1}, {(0, 0): 1}),
    3: ({(0, 0): 1}, {(0, 1): 1, (1, 1): -1}),
    4: ({(1, 1): 1}, {(1, 0): 1, (0, 0): -1}),
    5: ({(0, 0): 1, (0, 1): 1}, {(1, 1): 1}),
    6: ({(1, 0): 1, (0, 0): -1}, {(0, 0): 1, (0, 1): 1}),
    7: ({(0, 1): 1, (1, 1): -1}, {(1, 0): 1, (1, 1): 1}),
}
RESULT = {(0, 0): {1: 1, 4: 1, 5: -1, 7: 1}, (0, 1): {3: 1, 5: 1},
          (1, 0): {2: 1, 4: 1}, (1, 1): {1: 1, 2: -1, 3: 1, 6: 1}}
NESTED = (2, 3, 4, 5)
ORDER = (None, (1, 4), (0, 2), (0, 1), None, (1, 2), (0, 4), (1, 1),
         (0, 5), (0, 7), (1, 5), (1, 7), (1, 3), (0, 3), (1, 6), (0, 6))
GROUP_WORK = 16 + 2 * (7 * 8 - len(NESTED))

RING = 9
DELAY = 34
W_FROM = 246
W_PHASE = 10
WIDE = 6
READ_ORDER = tuple(24 * i + -j % 24 for j in range(24) for i in range(6))


def _combine(terms):
    terms = list(terms)
    acc = terms.pop(next(k for k, (c, _) in enumerate(terms) if c > 0))[1]
    for c, v in terms:
        acc = acc + v if c > 0 else acc - v
    return acc


def _pack_rows(v):
    n = v.shape[0] // 16
    v = v.reshape(n, 2, 8, v.shape[1])
    return pltpu.pack_elementwise([v[:, h].reshape(8 * n, -1) for h in range(2)], packed_dtype=BF16)


def _prune_packed(u):
    mate = lax.broadcasted_iota(jnp.int32, u.shape, 0) ^ 1
    lo = pltpu.bitcast((u << 16) & 0x7FFFFFFF, F32)
    hi = pltpu.bitcast(u & 0x7FFF0000, F32)
    big, small = jnp.maximum(lo, hi), jnp.minimum(lo, hi)
    nbig = jnp.take_along_axis(big, mate, axis=0, mode="promise_in_bounds")
    nsmall = jnp.take_along_axis(small, mate, axis=0, mode="promise_in_bounds")
    thr = jnp.maximum(jnp.minimum(big, nbig), jnp.maximum(small, nsmall))
    return u & (jnp.where(lo < thr, 0, 0xFFFF) | jnp.where(hi < thr, 0, -65536))


def _weight_forms():
    tall, short = {}, {}
    for g in range(2):
        tile = lambda k, s: 2 * k + s if 2 * k + s < 3 else 3 + g
        for m, (a, _) in STRASSEN.items():
            if m in NESTED:
                for n, (a2, _) in STRASSEN.items():
                    short[g, m, n] = tuple(sorted(
                        ((2 * i + i2, tile(k, s)), c * c2)
                        for (i, k), c in a.items() for (i2, s), c2 in a2.items()))
            else:
                for s in range(2):
                    tall[g, m, s] = tuple(sorted(((2 * i, tile(k, s)), c) for (i, k), c in a.items()))
    for q in range(4):
        short["E", q] = (((q, 5), 1),)
    return tall, short


def _distinct(forms):
    return list(dict.fromkeys(forms.values()))


def _prepare_weights(wbuf, tall_ref, short_ref):
    D, F = wbuf.shape
    u = pltpu.bitcast(wbuf[...], jnp.int32)
    rows = [_pack_rows(pltpu.bitcast(_prune_packed(u[8 * i:8 * i + 8]), BF16).astype(F32))
            for i in range(D // 16)]
    rows = rows[:32] + rows[24:28] + rows[32:36] + rows[28:36]
    a = pltpu.bitcast(pltpu.bitcast(jnp.concatenate(rows, axis=0), BF16).T, U32)
    where = {}
    for forms, ref in zip(_weight_forms(), (tall_ref, short_ref)):
        n = ref.shape[1]
        block = lambda q, t: a[q * F // 8:q * F // 8 + n, t * 128:(t + 1) * 128]
        for slot, form in enumerate(_distinct(forms)):
            if len(form) == 1:
                ref[slot] = block(*form[0][0])
            else:
                ref[slot] = pltpu.pack_elementwise([_combine(
                    (c, pltpu.unpack_elementwise(block(q, t), index=h, packed_dtype=BF16, unpacked_dtype=F32))
                    for (q, t), c in form) for h in range(2)], packed_dtype=BF16)
        where.update({name: (ref, _distinct(forms).index(form)) for name, form in forms.items()})
    return lambda *name: pltpu.bitcast(where[name][0][where[name][1]], BF16)


def _group(load, weights, bias_ref, store, progress):
    Q = bias_ref.shape[0] // 4
    loaded, prods, shared, stored, arrival = {}, {}, {}, set(), []

    def x_blocks(k, n, pair, h):
        if (k, n, pair) not in loaded:
            words = load(k, n, pair).reshape(64 * n, 128)
            loaded[k, n, pair] = pltpu.bitcast(words, BF16).astype(F32).reshape(8 * n, 2, 8, 128)
        return loaded[k, n, pair][:, h].reshape(64 * n, 128)

    def x_tile(g, t, j, h):
        if t < 3:
            return x_blocks(2 * t, 2, 2 * g + j, h)
        diff = x_blocks(7 + g, 1, 2 * g + j, h) - x_blocks(7 + g, 1, 2 * (1 - g) + j, h)
        return jnp.concatenate([x_blocks(6, 1, 2 * g + j, h), diff], axis=0)

    def dot(a, b):
        return jnp.dot(a, pltpu.bitcast(_pack_rows(b), BF16), preferred_element_type=F32)

    e_todo = [(2 * i + q, j, h) for i, j in ((1, 0), (0, 0), (0, 1), (1, 1))
              for h in range(2) for q in range(2)]

    def shared_pass():
        q, j, h = e_todo.pop(0)
        rhs = jnp.concatenate([x_blocks(7, 1, 2 + j, h), x_blocks(8, 1, j, h)], axis=0)
        shared[q, j, h] = dot(weights("E", q), rhs) + bias_ref[pl.ds(q * Q, Q)]
        arrival.append(("E", q // 2, j))
        progress(1)

    def product(g, m):
        operand = lambda s, h: _combine(
            (c, x_tile(g, 2 * k + s, j, h)) for (k, j), c in STRASSEN[m][1].items())
        if m in NESTED:
            mm = lambda n: dot(weights(g, m, n), _combine(
                (c, operand(s, h)) for (s, h), c in STRASSEN[n][1].items()))
            n5, n1, n4, n7 = mm(5), mm(1), mm(4), mm(7)
            c11 = (n1 + n4) + (n7 - n5)
            progress(4)
            n2, n3, n6 = mm(2), mm(3), mm(6)
            shared_pass()
            progress(3)
            prods[g, m] = (jnp.concatenate([c11, n2 + n4], axis=0),
                           jnp.concatenate([n3 + n5, n6 + (n3 - n2) + n1], axis=0))
        else:
            p = [dot(weights(g, m, s), operand(s, h)) for h in range(2) for s in range(2)]
            prods[g, m] = (p[0] + p[1], p[2] + p[3])
            progress(8)
        arrival.append((g, m))

    def finish(g, i, j):
        values = []
        for h in range(2):
            terms = {(g, m): (c, prods[g, m][h]) for m, c in RESULT[i, j].items()}
            terms["E", i, j] = (1, jnp.concatenate([shared[2 * i + q, j, h] for q in range(2)], axis=0))
            values.append(_combine(terms[k] for k in sorted(terms, key=arrival[::-1].index)))
        store(i, 2 * g + j, values)

    for step in ORDER:
        if step is None:
            for _ in range(4):
                shared_pass()
        else:
            product(*step)
        loaded.clear()
        for g in range(2):
            for (i, j), ms in RESULT.items():
                if ((g, i, j) not in stored and all((g, m) in prods for m in ms)
                        and (2 * i + 1, j, 1) in shared):
                    finish(g, i, j)
                    stored.add((g, i, j))
    assert len(stored) == 8


def _kernel(x_hbm, w_hbm, b_hbm, o_hbm, xbuf, obuf, wbuf, bbuf, tall_ref, short_ref, bias_ref,
            xsem, first_sem, osem):
    F = w_hbm.shape[1]
    B = obuf.shape[0]
    x_words = x_hbm.bitcast(U32)
    o_wide, obuf_wide = (r.reshape(B // 2, 9, 16, 16, 16, 128) for r in (o_hbm, obuf))

    def read_first(u):
        for r in range(8):
            at = (0, slice(None), r, pl.ds(4 * u, 4))
            pltpu.make_async_copy(x_words.at[at], xbuf.at[at], first_sem.at[min(u, 2)]).start(priority=1)

    def read(b, slot, k):
        g = READ_ORDER[k]
        at = (g >> 4, (g >> 1) & 7, pl.ds(8 * (g & 1), 8))
        pltpu.make_async_copy(x_words.at[(b, *at)], xbuf.at[(slot, *at)], xsem.at[slot]).start(priority=k % 2)

    def arrived(groups, sem):
        part = xbuf.at[0, :, :, pl.ds(0, 4 * groups)]
        pltpu.make_async_copy(part, part, sem).wait()

    def write(b, r, q):
        at = (b, slice(None), r, pl.ds(2 * q, 2))
        pltpu.make_async_copy(obuf.at[at], o_hbm.at[at], osem.at[0]).start()

    def write_wide(n):
        for q in range(2):
            at = (n >> 5, slice(None), (n >> 1) & 15, pl.ds(8 * (n & 1) + 4 * q, 4))
            pltpu.make_async_copy(obuf_wide.at[at], o_wide.at[at], osem.at[0]).start()

    def write_narrow(n):
        for q in range(4):
            write(n >> 4, 2 * (n & 3) + ((n >> 2) & 1), ((n >> 1) & 4) + q)

    def write_group(u):
        for r in range(8):
            for q in range(2):
                write(B - 1, r, 2 * u + q)

    params = [pltpu.make_async_copy(b_hbm, bbuf, first_sem.at[3]),
              pltpu.make_async_copy(w_hbm, wbuf, first_sem.at[4])]
    for copy in params:
        copy.start()
    read_first(0)
    read_first(1)
    for copy in params:
        copy.wait()
    read_first(2)
    read_first(3)
    weights = _prepare_weights(wbuf, tall_ref, short_ref)
    bias_ref[...] = jnp.broadcast_to(bbuf[...].reshape(1, F).astype(F32), (128, F)).T

    wrap = lambda s: jnp.where(s >= RING, s - RING, s)

    def half_batch(t, carry):
        slot, read_slot, written = carry
        pl.when(t == 0)(lambda: arrived(1, first_sem.at[0]))
        pl.when(t == 1)(lambda: arrived(2, first_sem.at[2]))
        pl.when(jnp.logical_and(t > 1, t & 1 == 0))(lambda: arrived(4, xsem.at[slot]))
        read_slots = (read_slot, wrap(read_slot + 1))
        work = 0

        def progress(n):
            nonlocal work, written
            before, work = work, work + n
            per = len(READ_ORDER)
            due = range(*(per - DELAY + v * per // (2 * GROUP_WORK) for v in (before, work)))
            for h in range(2):
                ks = [k - h * per for k in due if k // per == h]
                if ks:
                    @pl.when(jnp.logical_and(t + h > 0, t + h < B))
                    def _():
                        for k in ks:
                            read(t + h, read_slots[h], k)
            for k in range(*(pl.cdiv((v - W_PHASE) * 8, GROUP_WORK) for v in (before, work))):
                wide = written < 32 * WIDE
                ready = jnp.where(wide, written | 31, written) < 8 * t
                go = jnp.logical_and(16 * t + k >= W_FROM, ready)
                pl.when(jnp.logical_and(go, wide))(lambda: write_wide(written))
                pl.when(jnp.logical_and(go, jnp.logical_not(wide)))(lambda: write_narrow(written))
                written = written + go.astype(jnp.int32)
            if before < GROUP_WORK * 6 // 5 <= work:
                pl.when(t == 2 * B - 1)(lambda: write_group(2))

        for u in range(2):
            first = (t & 1) * 8 + 4 * u

            def load(k, n, pair):
                return xbuf[slot, pl.ds(k, n), :, first + pair]

            def store(i, pair, values):
                v = jnp.concatenate([a.reshape(36, 8, 128) for a in values], axis=1).astype(obuf.dtype)
                whole, part = (v[:32], v[32:]) if i == 0 else (v[4:], v[:4])
                obuf[t >> 1, pl.ds(5 * i, 4), :, first + pair] = whole.reshape(4, 8, 16, 128)
                obuf[t >> 1, 4, pl.ds(4 * i, 4), first + pair] = part

            if u:
                pl.when(t == 0)(lambda: arrived(1, first_sem.at[1]))
            _group(load, weights, bias_ref, store, progress)
        return wrap(slot + (t & 1)), read_slots[1], written

    _, _, written = lax.fori_loop(0, 2 * B, half_batch, (0, 0, 0))
    lax.fori_loop(written, 8 * (2 * B - 1), lambda n, _: write_narrow(n), None)
    write_group(3)
    pltpu.make_async_copy(obuf, obuf, osem.at[0]).wait()


@jax.jit
def pallas_standalone__structured_sparse_n_m__ragged_kernel(
    x: jax.Array,
    w: jax.Array,
    b: jax.Array,
):
    B, S, D = x.shape
    F = w.shape[1]
    assert (B, S, D, F) == (16, 4096, 576, 576)
    tall, short = _weight_forms()
    xt = jnp.transpose(x.reshape(B, 32, 128, 9, 8, 8), (0, 3, 4, 1, 5, 2)).reshape(B, 9, 8, 16, 16, 128)
    out = pl.pallas_call(
        _kernel,
        in_specs=[pl.BlockSpec(memory_space=pl.ANY)] * 3,
        out_specs=pl.BlockSpec(memory_space=pl.ANY),
        out_shape=jax.ShapeDtypeStruct(xt.shape, x.dtype),
        scratch_shapes=[
            pltpu.VMEM((RING, 9, 8, 16, 8, 128), U32),
            pltpu.VMEM(xt.shape, x.dtype),
            pltpu.VMEM((D, F), w.dtype),
            pltpu.VMEM((F,), b.dtype),
            pltpu.VMEM((len(_distinct(tall)), F // 4, 128), U32),
            pltpu.VMEM((len(_distinct(short)), F // 8, 128), U32),
            pltpu.VMEM((F, 128), F32),
            pltpu.SemaphoreType.DMA((RING,)),
            pltpu.SemaphoreType.DMA((5,)),
            pltpu.SemaphoreType.DMA((1,)),
        ],
        compiler_params=pltpu.CompilerParams(
            vmem_limit_bytes=128 * 1024 * 1024,
            disable_bounds_checks=True,
            disable_semaphore_checks=True,
            flags={"XLA_TPU_RESCHEDULE_DMA_DONES": True},
        ),
    )(xt, w, b)
    return jnp.transpose(out.reshape(B, 9, 8, 32, 8, 128), (0, 3, 5, 1, 2, 4)).reshape(B, S, F)
```

```python
import jax
import jax.numpy as jnp
from jax import lax
import jax.experimental.pallas as pl
import jax.experimental.pallas.tpu as pltpu

F32, BF16, U32 = jnp.float32, jnp.bfloat16, jnp.uint32

STRASSEN = {
    1: ({(0, 0): 1, (1, 1): 1}, {(0, 0): 1, (1, 1): 1}),
    2: ({(1, 0): 1, (1, 1): 1}, {(0, 0): 1}),
    3: ({(0, 0): 1}, {(0, 1): 1, (1, 1): -1}),
    4: ({(1, 1): 1}, {(1, 0): 1, (0, 0): -1}),
    5: ({(0, 0): 1, (0, 1): 1}, {(1, 1): 1}),
    6: ({(1, 0): 1, (0, 0): -1}, {(0, 0): 1, (0, 1): 1}),
    7: ({(0, 1): 1, (1, 1): -1}, {(1, 0): 1, (1, 1): 1}),
}
RESULT = {(0, 0): {1: 1, 4: 1, 5: -1, 7: 1}, (0, 1): {3: 1, 5: 1},
          (1, 0): {2: 1, 4: 1}, (1, 1): {1: 1, 2: -1, 3: 1, 6: 1}}
NESTED = (2, 3, 4, 5)
ORDER = (None, (1, 4), (0, 2), (0, 1), None, (1, 2), (0, 4), (1, 1),
         (0, 5), (0, 7), (1, 5), (1, 7), (1, 3), (0, 3), (1, 6), (0, 6))
GROUP_WORK = 16 + 2 * (7 * 8 - len(NESTED))

RING = 9
DELAY = 50
W_FROM = 249
W_PHASE = 0
READ_ORDER = tuple(24 * i + -j % 24 for j in range(24) for i in range(6))


def _combine(terms):
    terms = list(terms)
    acc = terms.pop(next(k for k, (c, _) in enumerate(terms) if c > 0))[1]
    for c, v in terms:
        acc = acc + v if c > 0 else acc - v
    return acc


def _pack_rows(v):
    n = v.shape[0] // 16
    v = v.reshape(n, 2, 8, v.shape[1])
    return pltpu.pack_elementwise([v[:, h].reshape(8 * n, -1) for h in range(2)], packed_dtype=BF16)


def _prune_packed(u):
    mate = lax.broadcasted_iota(jnp.int32, u.shape, 0) ^ 1
    lo = pltpu.bitcast((u << 16) & 0x7FFFFFFF, F32)
    hi = pltpu.bitcast(u & 0x7FFF0000, F32)
    big, small = jnp.maximum(lo, hi), jnp.minimum(lo, hi)
    nbig = jnp.take_along_axis(big, mate, axis=0, mode="promise_in_bounds")
    nsmall = jnp.take_along_axis(small, mate, axis=0, mode="promise_in_bounds")
    thr = jnp.maximum(jnp.minimum(big, nbig), jnp.maximum(small, nsmall))
    return u & (jnp.where(lo < thr, 0, 0xFFFF) | jnp.where(hi < thr, 0, -65536))


def _weight_forms():
    tall, short = {}, {}
    for g in range(2):
        tile = lambda k, s: 2 * k + s if 2 * k + s < 3 else 3 + g
        for m, (a, _) in STRASSEN.items():
            if m in NESTED:
                for n, (a2, _) in STRASSEN.items():
                    short[g, m, n] = tuple(sorted(
                        ((2 * i + i2, tile(k, s)), c * c2)
                        for (i, k), c in a.items() for (i2, s), c2 in a2.items()))
            else:
                for s in range(2):
                    tall[g, m, s] = tuple(sorted(((2 * i, tile(k, s)), c) for (i, k), c in a.items()))
    for q in range(4):
        short["E", q] = (((q, 5), 1),)
    return tall, short


def _distinct(forms):
    return list(dict.fromkeys(forms.values()))


def _prepare_weights(wbuf, tall_ref, short_ref):
    D, F = wbuf.shape
    u = pltpu.bitcast(wbuf[...], jnp.int32)
    rows = [_pack_rows(pltpu.bitcast(_prune_packed(u[8 * i:8 * i + 8]), BF16).astype(F32))
            for i in range(D // 16)]
    rows = rows[:32] + rows[24:28] + rows[32:36] + rows[28:36]
    a = pltpu.bitcast(pltpu.bitcast(jnp.concatenate(rows, axis=0), BF16).T, U32)
    where = {}
    for forms, ref in zip(_weight_forms(), (tall_ref, short_ref)):
        n = ref.shape[1]
        block = lambda q, t: a[q * F // 8:q * F // 8 + n, t * 128:(t + 1) * 128]
        for slot, form in enumerate(_distinct(forms)):
            if len(form) == 1:
                ref[slot] = block(*form[0][0])
            else:
                ref[slot] = pltpu.pack_elementwise([_combine(
                    (c, pltpu.unpack_elementwise(block(q, t), index=h, packed_dtype=BF16, unpacked_dtype=F32))
                    for (q, t), c in form) for h in range(2)], packed_dtype=BF16)
        where.update({name: (ref, _distinct(forms).index(form)) for name, form in forms.items()})
    return lambda *name: pltpu.bitcast(where[name][0][where[name][1]], BF16)


def _group(load, weights, bias_ref, store, progress):
    Q = bias_ref.shape[0] // 4
    loaded, prods, shared, stored, arrival = {}, {}, {}, set(), []

    def x_blocks(k, n, pair, h):
        if (k, n, pair) not in loaded:
            words = load(k, n, pair).reshape(64 * n, 128)
            loaded[k, n, pair] = pltpu.bitcast(words, BF16).astype(F32).reshape(8 * n, 2, 8, 128)
        return loaded[k, n, pair][:, h].reshape(64 * n, 128)

    def x_tile(g, t, j, h):
        if t < 3:
            return x_blocks(2 * t, 2, 2 * g + j, h)
        diff = x_blocks(7 + g, 1, 2 * g + j, h) - x_blocks(7 + g, 1, 2 * (1 - g) + j, h)
        return jnp.concatenate([x_blocks(6, 1, 2 * g + j, h), diff], axis=0)

    def dot(a, b):
        return jnp.dot(a, pltpu.bitcast(_pack_rows(b), BF16), preferred_element_type=F32)

    e_todo = [(2 * i + q, j, h) for i, j in ((1, 0), (0, 0), (0, 1), (1, 1))
              for h in range(2) for q in range(2)]

    def shared_pass():
        q, j, h = e_todo.pop(0)
        rhs = jnp.concatenate([x_blocks(7, 1, 2 + j, h), x_blocks(8, 1, j, h)], axis=0)
        shared[q, j, h] = dot(weights("E", q), rhs) + bias_ref[pl.ds(q * Q, Q)]
        arrival.append(("E", q // 2, j))
        progress(1)

    def product(g, m):
        operand = lambda s, h: _combine(
            (c, x_tile(g, 2 * k + s, j, h)) for (k, j), c in STRASSEN[m][1].items())
        if m in NESTED:
            mm = lambda n: dot(weights(g, m, n), _combine(
                (c, operand(s, h)) for (s, h), c in STRASSEN[n][1].items()))
            n5, n1, n4, n7 = mm(5), mm(1), mm(4), mm(7)
            c11 = (n1 + n4) + (n7 - n5)
            progress(4)
            n2, n3, n6 = mm(2), mm(3), mm(6)
            shared_pass()
            progress(3)
            prods[g, m] = (jnp.concatenate([c11, n2 + n4], axis=0),
                           jnp.concatenate([n3 + n5, n6 + (n3 - n2) + n1], axis=0))
        else:
            p = [dot(weights(g, m, s), operand(s, h)) for h in range(2) for s in range(2)]
            prods[g, m] = (p[0] + p[1], p[2] + p[3])
            progress(8)
        arrival.append((g, m))

    def finish(g, i, j):
        values = []
        for h in range(2):
            terms = {(g, m): (c, prods[g, m][h]) for m, c in RESULT[i, j].items()}
            terms["E", i, j] = (1, jnp.concatenate([shared[2 * i + q, j, h] for q in range(2)], axis=0))
            values.append(_combine(terms[k] for k in sorted(terms, key=arrival[::-1].index)))
        store(i, 2 * g + j, values)

    for step in ORDER:
        if step is None:
            for _ in range(4):
                shared_pass()
        else:
            product(*step)
        loaded.clear()
        for g in range(2):
            for (i, j), ms in RESULT.items():
                if ((g, i, j) not in stored and all((g, m) in prods for m in ms)
                        and (2 * i + 1, j, 1) in shared):
                    finish(g, i, j)
                    stored.add((g, i, j))
    assert len(stored) == 8


def _kernel(x_hbm, w_hbm, b_hbm, o_hbm, xbuf, obuf, wbuf, bbuf, tall_ref, short_ref, bias_ref,
            xsem, first_sem, osem):
    F = w_hbm.shape[1]
    B = obuf.shape[0]
    x_words = x_hbm.bitcast(U32)
    o_wide, obuf_wide = (r.reshape(B // 2, 9, 16, 16, 16, 128) for r in (o_hbm, obuf))
    wrap = lambda s: jnp.where(s >= RING, s - RING, s)

    def read_first(u):
        for r in range(8):
            at = (0, slice(None), r, pl.ds(4 * u, 4))
            pltpu.make_async_copy(x_words.at[at], xbuf.at[at], first_sem.at[u]).start(priority=1)

    def read(b, slot, k):
        g = READ_ORDER[k]
        at = (g >> 4, (g >> 1) & 7, pl.ds(8 * (g & 1), 8))
        pltpu.make_async_copy(x_words.at[(b, *at)], xbuf.at[(slot, *at)], xsem.at[slot]).start(priority=k % 2)

    def arrived(part, sem):
        pltpu.make_async_copy(part, part, sem).wait()

    def write_wide(p, n):
        for q in range(2):
            at = (p, slice(None), n >> 1, pl.ds(8 * (n & 1) + 4 * q, 4))
            pltpu.make_async_copy(obuf_wide.at[at], o_wide.at[at], osem.at[0]).start()

    def write(b, r, quarters):
        for q in quarters:
            at = (b, slice(None), r, pl.ds(2 * q, 2))
            pltpu.make_async_copy(obuf.at[at], o_hbm.at[at], osem.at[0]).start()

    params = [pltpu.make_async_copy(b_hbm, bbuf, first_sem.at[4]),
              pltpu.make_async_copy(w_hbm, wbuf, first_sem.at[5])]
    for copy in params:
        copy.start()
    read_first(0)
    read_first(1)
    for copy in params:
        copy.wait()
    read_first(2)
    read_first(3)
    weights = _prepare_weights(wbuf, tall_ref, short_ref)
    bias_ref[...] = jnp.broadcast_to(bbuf[...].reshape(1, F).astype(F32), (128, F)).T

    def batch(t, _):
        slot = wrap(t)
        pl.when(t > 0)(lambda: arrived(xbuf.at[slot], xsem.at[slot]))
        slots = [wrap(2 * t + e) for e in range(3)]
        work = 0

        def progress(n):
            nonlocal work
            before, work = work, work + n
            per = len(READ_ORDER)
            due = range(*(per - DELAY + v * per // (2 * GROUP_WORK) for v in (before, work)))
            for e in range(3):
                ks = [k % per for k in due if k // per == e]
                if ks:
                    @pl.when(jnp.logical_and(2 * t + e > 0, 2 * t + e < B))
                    def _():
                        for k in ks:
                            read(2 * t + e, slots[e], k)
            for k in range(*(pl.cdiv((v - W_PHASE) * 8, GROUP_WORK) for v in (before, work))):
                dp, n = divmod(k - W_FROM, 32)
                pl.when(jnp.logical_and(t + dp >= 0, t + dp < B // 2 - 2))(lambda: write_wide(t + dp, n))
                pl.when(t == B - 2)(lambda: write_wide(B // 2 - 2, k))
                if k < 16:
                    pl.when(t == B - 1)(lambda: write(B - 2, k >> 1, range(4 * (k & 1), 4 * (k & 1) + 4)))
                elif 17 <= k < 25:
                    pl.when(t == B - 1)(lambda: write(B - 1, 2 * (k - 17) % 8 + (k - 17) // 4, range(4)))
                elif 25 <= k < 29:
                    @pl.when(t == B - 1)
                    def _():
                        for r in (2 * (k - 25), 2 * (k - 25) + 1):
                            write(B - 1, r, (4, 5))

        for u in range(4):
            def load(k, n, pair):
                return xbuf[slot, pl.ds(k, n), :, 4 * u + pair]

            def store(i, pair, values):
                v = jnp.concatenate([a.reshape(36, 8, 128) for a in values], axis=1).astype(obuf.dtype)
                whole, part = (v[:32], v[32:]) if i == 0 else (v[4:], v[:4])
                obuf[t, pl.ds(5 * i, 4), :, 4 * u + pair] = whole.reshape(4, 8, 16, 128)
                obuf[t, 4, pl.ds(4 * i, 4), 4 * u + pair] = part

            pl.when(t == 0)(lambda: arrived(xbuf.at[0, :, :, pl.ds(4 * u, 4)], first_sem.at[u]))
            _group(load, weights, bias_ref, store, progress)

    assert W_FROM >= 32 * (B // 2 - 1)
    lax.fori_loop(0, B, batch, None)
    for r in range(8):
        write(B - 1, r, (6, 7))
    pltpu.make_async_copy(obuf, obuf, osem.at[0]).wait()


@jax.jit
def pallas_standalone__structured_sparse_n_m__ragged_kernel(
    x: jax.Array,
    w: jax.Array,
    b: jax.Array,
):
    B, S, D = x.shape
    F = w.shape[1]
    assert (B, S, D, F) == (16, 4096, 576, 576)
    tall, short = _weight_forms()
    xt = jnp.transpose(x.reshape(B, 32, 128, 9, 8, 8), (0, 3, 4, 1, 5, 2)).reshape(B, 9, 8, 16, 16, 128)
    out = pl.pallas_call(
        _kernel,
        in_specs=[pl.BlockSpec(memory_space=pl.ANY)] * 3,
        out_specs=pl.BlockSpec(memory_space=pl.ANY),
        out_shape=jax.ShapeDtypeStruct(xt.shape, x.dtype),
        scratch_shapes=[
            pltpu.VMEM((RING, 9, 8, 16, 8, 128), U32),
            pltpu.VMEM(xt.shape, x.dtype),
            pltpu.VMEM((D, F), w.dtype),
            pltpu.VMEM((F,), b.dtype),
            pltpu.VMEM((len(_distinct(tall)), F // 4, 128), U32),
            pltpu.VMEM((len(_distinct(short)), F // 8, 128), U32),
            pltpu.VMEM((F, 128), F32),
            pltpu.SemaphoreType.DMA((RING,)),
            pltpu.SemaphoreType.DMA((6,)),
            pltpu.SemaphoreType.DMA((1,)),
        ],
        compiler_params=pltpu.CompilerParams(
            vmem_limit_bytes=128 * 1024 * 1024,
            disable_bounds_checks=True,
            disable_semaphore_checks=True,
            flags={"XLA_TPU_RESCHEDULE_DMA_DONES": True},
        ),
    )(xt, w, b)
    return jnp.transpose(out.reshape(B, 9, 8, 32, 8, 128), (0, 3, 5, 1, 2, 4)).reshape(B, S, F)
```

```python
import jax
import jax.numpy as jnp
from jax import lax
import jax.experimental.pallas as pl
import jax.experimental.pallas.tpu as pltpu

F32, BF16, U32 = jnp.float32, jnp.bfloat16, jnp.uint32

STRASSEN = {
    1: ({(0, 0): 1, (1, 1): 1}, {(0, 0): 1, (1, 1): 1}),
    2: ({(1, 0): 1, (1, 1): 1}, {(0, 0): 1}),
    3: ({(0, 0): 1}, {(0, 1): 1, (1, 1): -1}),
    4: ({(1, 1): 1}, {(1, 0): 1, (0, 0): -1}),
    5: ({(0, 0): 1, (0, 1): 1}, {(1, 1): 1}),
    6: ({(1, 0): 1, (0, 0): -1}, {(0, 0): 1, (0, 1): 1}),
    7: ({(0, 1): 1, (1, 1): -1}, {(1, 0): 1, (1, 1): 1}),
}
RESULT = {(0, 0): {1: 1, 4: 1, 5: -1, 7: 1}, (0, 1): {3: 1, 5: 1},
          (1, 0): {2: 1, 4: 1}, (1, 1): {1: 1, 2: -1, 3: 1, 6: 1}}
NESTED = (2, 3, 4, 5)
ORDER = (None, (1, 4), (0, 2), (0, 1), None, (1, 2), (0, 4), (1, 1),
         (0, 5), (0, 7), (1, 5), (1, 7), (1, 3), (0, 3), (1, 6), (0, 6))
GROUP_WORK = 16 + 2 * (7 * 8 - len(NESTED))

RING = 9
DELAY = 50
W_FROM = 248
READ_ORDER = tuple(24 * i + -j % 24 for j in range(24) for i in range(6))


def _combine(terms):
    terms = list(terms)
    acc = terms.pop(next(k for k, (c, _) in enumerate(terms) if c > 0))[1]
    for c, v in terms:
        acc = acc + v if c > 0 else acc - v
    return acc


def _pack_rows(v):
    n = v.shape[0] // 16
    v = v.reshape(n, 2, 8, v.shape[1])
    return pltpu.pack_elementwise([v[:, h].reshape(8 * n, -1) for h in range(2)], packed_dtype=BF16)


def _prune_packed(u):
    mate = lax.broadcasted_iota(jnp.int32, u.shape, 0) ^ 1
    lo = pltpu.bitcast((u << 16) & 0x7FFFFFFF, F32)
    hi = pltpu.bitcast(u & 0x7FFF0000, F32)
    big, small = jnp.maximum(lo, hi), jnp.minimum(lo, hi)
    nbig = jnp.take_along_axis(big, mate, axis=0, mode="promise_in_bounds")
    nsmall = jnp.take_along_axis(small, mate, axis=0, mode="promise_in_bounds")
    thr = jnp.maximum(jnp.minimum(big, nbig), jnp.maximum(small, nsmall))
    return u & (jnp.where(lo < thr, 0, 0xFFFF) | jnp.where(hi < thr, 0, -65536))


def _weight_forms():
    tall, short = {}, {}
    for g in range(2):
        tile = lambda k, s: 2 * k + s if 2 * k + s < 3 else 3 + g
        for m, (a, _) in STRASSEN.items():
            if m in NESTED:
                for n, (a2, _) in STRASSEN.items():
                    short[g, m, n] = tuple(sorted(
                        ((2 * i + i2, tile(k, s)), c * c2)
                        for (i, k), c in a.items() for (i2, s), c2 in a2.items()))
            else:
                for s in range(2):
                    tall[g, m, s] = tuple(sorted(((2 * i, tile(k, s)), c) for (i, k), c in a.items()))
    for q in range(4):
        short["E", q] = (((q, 5), 1),)
    return tall, short


def _distinct(forms):
    return list(dict.fromkeys(forms.values()))


def _prepare_weights(wbuf, tall_ref, short_ref):
    D, F = wbuf.shape
    u = pltpu.bitcast(wbuf[...], jnp.int32)
    rows = [_pack_rows(pltpu.bitcast(_prune_packed(u[8 * i:8 * i + 8]), BF16).astype(F32))
            for i in range(D // 16)]
    rows = rows[:32] + rows[24:28] + rows[32:36] + rows[28:36]
    a = pltpu.bitcast(pltpu.bitcast(jnp.concatenate(rows, axis=0), BF16).T, U32)
    where = {}
    for forms, ref in zip(_weight_forms(), (tall_ref, short_ref)):
        n = ref.shape[1]
        block = lambda q, t: a[q * F // 8:q * F // 8 + n, t * 128:(t + 1) * 128]
        for slot, form in enumerate(_distinct(forms)):
            if len(form) == 1:
                ref[slot] = block(*form[0][0])
            else:
                ref[slot] = pltpu.pack_elementwise([_combine(
                    (c, pltpu.unpack_elementwise(block(q, t), index=h, packed_dtype=BF16, unpacked_dtype=F32))
                    for (q, t), c in form) for h in range(2)], packed_dtype=BF16)
        where.update({name: (ref, _distinct(forms).index(form)) for name, form in forms.items()})
    return lambda *name: pltpu.bitcast(where[name][0][where[name][1]], BF16)


def _group(load, weights, bias_ref, store, progress):
    Q = bias_ref.shape[0] // 4
    loaded, prods, shared, stored, arrival = {}, {}, {}, set(), []

    def x_blocks(k, n, pair, h):
        if (k, n, pair) not in loaded:
            loaded[k, n, pair] = load(k, n, pair).astype(F32).reshape(8 * n, 2, 8, 128)
        return loaded[k, n, pair][:, h].reshape(64 * n, 128)

    def x_tile(g, t, j, h):
        if t < 3:
            return x_blocks(2 * t, 2, 2 * g + j, h)
        diff = x_blocks(7 + g, 1, 2 * g + j, h) - x_blocks(7 + g, 1, 2 * (1 - g) + j, h)
        return jnp.concatenate([x_blocks(6, 1, 2 * g + j, h), diff], axis=0)

    def dot(a, b):
        return jnp.dot(a, pltpu.bitcast(_pack_rows(b), BF16), preferred_element_type=F32)

    e_todo = [(2 * i + q, j, h) for i, j in ((1, 0), (0, 0), (0, 1), (1, 1))
              for h in range(2) for q in range(2)]

    def shared_pass():
        q, j, h = e_todo.pop(0)
        rhs = jnp.concatenate([x_blocks(7, 1, 2 + j, h), x_blocks(8, 1, j, h)], axis=0)
        shared[q, j, h] = dot(weights("E", q), rhs) + bias_ref[pl.ds(q * Q, Q)]
        arrival.append(("E", q // 2, j))
        progress(1)

    def product(g, m):
        operand = lambda s, h: _combine(
            (c, x_tile(g, 2 * k + s, j, h)) for (k, j), c in STRASSEN[m][1].items())
        if m in NESTED:
            mm = lambda n: dot(weights(g, m, n), _combine(
                (c, operand(s, h)) for (s, h), c in STRASSEN[n][1].items()))
            n5, n1, n4, n7 = mm(5), mm(1), mm(4), mm(7)
            c11 = (n1 + n4) + (n7 - n5)
            progress(4)
            n2, n3, n6 = mm(2), mm(3), mm(6)
            shared_pass()
            progress(3)
            prods[g, m] = (jnp.concatenate([c11, n2 + n4], axis=0),
                           jnp.concatenate([n3 + n5, n6 + (n3 - n2) + n1], axis=0))
        else:
            p = [dot(weights(g, m, s), operand(s, h)) for h in range(2) for s in range(2)]
            prods[g, m] = (p[0] + p[1], p[2] + p[3])
            progress(8)
        arrival.append((g, m))

    def finish(g, i, j):
        values = []
        for h in range(2):
            terms = {(g, m): (c, prods[g, m][h]) for m, c in RESULT[i, j].items()}
            terms["E", i, j] = (1, jnp.concatenate([shared[2 * i + q, j, h] for q in range(2)], axis=0))
            values.append(_combine(terms[k] for k in sorted(terms, key=arrival[::-1].index)))
        store(i, 2 * g + j, values)

    for step in ORDER:
        if step is None:
            for _ in range(4):
                shared_pass()
        else:
            product(*step)
        loaded.clear()
        for g in range(2):
            for (i, j), ms in RESULT.items():
                if ((g, i, j) not in stored and all((g, m) in prods for m in ms)
                        and (2 * i + 1, j, 1) in shared):
                    finish(g, i, j)
                    stored.add((g, i, j))
    assert len(stored) == 8


def _kernel(x_hbm, w_hbm, b_hbm, o_hbm, xbuf, obuf, wbuf, bbuf, tall_ref, short_ref, bias_ref,
            xsem, first_sem, osem):
    F = w_hbm.shape[1]
    B = obuf.shape[0]
    o_wide, obuf_wide = (r.reshape(B // 2, 9, 16, 16, 16, 128) for r in (o_hbm, obuf))
    wrap = lambda s: jnp.where(s >= RING, s - RING, s)

    def read(b, slot, at, sem, priority):
        pltpu.make_async_copy(x_hbm.at[(b, *at)], xbuf.at[(slot, *at)], sem).start(priority=priority)

    def finish(part, sem):
        pltpu.make_async_copy(part, part, sem).wait()

    def write_wide(p, n):
        at = (p, slice(None), n >> 1, pl.ds(8 * (n & 1), 8))
        pltpu.make_async_copy(obuf_wide.at[at], o_wide.at[at], osem.at[0]).start()

    def write_narrow(b, r, half):
        for q in range(4):
            at = (b, slice(None), r, pl.ds(8 * half + 2 * q, 2))
            pltpu.make_async_copy(obuf.at[at], o_hbm.at[at], osem.at[0]).start()

    even_then_odd = (0, 2, 4, 6, 1, 3, 5, 7)

    params = [pltpu.make_async_copy(b_hbm, bbuf, first_sem.at[3]),
              pltpu.make_async_copy(w_hbm, wbuf, first_sem.at[4])]
    for copy in params:
        copy.start()
    for u in range(2):
        for r in range(8):
            read(0, 0, (slice(None), r, pl.ds(4 * u, 4)), first_sem.at[u], 1)
    for copy in params:
        copy.wait()
    weights = _prepare_weights(wbuf, tall_ref, short_ref)
    bias_ref[...] = jnp.broadcast_to(bbuf[...].reshape(1, F).astype(F32), (128, F)).T

    def batch(t, _):
        slot = wrap(t)
        pl.when(t > 0)(lambda: finish(xbuf.at[slot], xsem.at[slot]))
        slots = [wrap(2 * t + e) for e in range(3)]
        work = 0

        def progress(n):
            nonlocal work
            span, work = (work, work + n), work + n
            per = len(READ_ORDER)
            due = range(*(per - DELAY + v * per // (2 * GROUP_WORK) for v in span))
            for e in range(3):
                ks = [k % per for k in due if k // per == e]
                if ks:
                    @pl.when(jnp.logical_and(2 * t + e > 0, 2 * t + e < B))
                    def _():
                        for k in ks:
                            g = READ_ORDER[k]
                            at = (g >> 4, (g >> 1) & 7, pl.ds(8 * (g & 1), 8))
                            read(2 * t + e, slots[e], at, xsem.at[slots[e]], k % 2)
            ks = range(*(min(72, v * 72 * per // (2 * GROUP_WORK * DELAY)) for v in span))
            if ks:
                @pl.when(t == 0)
                def _():
                    for k in ks:
                        read(0, 0, (k % 9, k // 9, pl.ds(8, 8)), first_sem.at[2], k % 2)
            for k in range(*(pl.cdiv(v * 8, GROUP_WORK) for v in span)):
                dp, n = divmod(k - W_FROM, 32)
                pl.when(jnp.logical_and(t + dp >= 0, t + dp < B // 2 - 2))(lambda: write_wide(t + dp, n))
                pl.when(t == B - 2)(lambda: write_wide(B // 2 - 2, k))
                if k < 16:
                    pl.when(t == B - 1)(lambda: write_narrow(B - 2, k >> 1, k & 1))
                elif 17 <= k < 25:
                    pl.when(t == B - 1)(lambda: write_narrow(B - 1, even_then_odd[k - 17], 0))

        for u in range(4):
            def load(k, n, pair):
                return xbuf[slot, pl.ds(k, n), :, 4 * u + pair]

            def store(i, pair, values):
                v = jnp.concatenate([a.reshape(36, 8, 128) for a in values], axis=1).astype(obuf.dtype)
                whole, part = (v[:32], v[32:]) if i == 0 else (v[4:], v[:4])
                obuf[t, pl.ds(5 * i, 4), :, 4 * u + pair] = whole.reshape(4, 8, 16, 128)
                obuf[t, 4, pl.ds(4 * i, 4), 4 * u + pair] = part

            if u < 3:
                part = xbuf.at[0, :, :, pl.ds(4 * u, 8 if u == 2 else 4)]
                pl.when(t == 0)(lambda: finish(part, first_sem.at[u]))
            _group(load, weights, bias_ref, store, progress)

    assert W_FROM >= 32 * (B // 2 - 1)
    lax.fori_loop(0, B, batch, None)
    for r in even_then_odd:
        write_narrow(B - 1, r, 1)
    finish(obuf, osem.at[0])


@jax.jit
def pallas_standalone__structured_sparse_n_m__ragged_kernel(
    x: jax.Array,
    w: jax.Array,
    b: jax.Array,
):
    B, S, D = x.shape
    F = w.shape[1]
    assert (B, S, D, F) == (16, 4096, 576, 576)
    tall, short = _weight_forms()
    xt = jnp.transpose(x.reshape(B, 32, 128, 9, 8, 8), (0, 3, 4, 1, 5, 2)).reshape(B, 9, 8, 16, 16, 128)
    out = pl.pallas_call(
        _kernel,
        in_specs=[pl.BlockSpec(memory_space=pl.ANY)] * 3,
        out_specs=pl.BlockSpec(memory_space=pl.ANY),
        out_shape=jax.ShapeDtypeStruct(xt.shape, x.dtype),
        scratch_shapes=[
            pltpu.VMEM((RING, *xt.shape[1:]), x.dtype),
            pltpu.VMEM(xt.shape, x.dtype),
            pltpu.VMEM((D, F), w.dtype),
            pltpu.VMEM((F,), b.dtype),
            pltpu.VMEM((len(_distinct(tall)), F // 4, 128), U32),
            pltpu.VMEM((len(_distinct(short)), F // 8, 128), U32),
            pltpu.VMEM((F, 128), F32),
            pltpu.SemaphoreType.DMA((RING,)),
            pltpu.SemaphoreType.DMA((5,)),
            pltpu.SemaphoreType.DMA((1,)),
        ],
        compiler_params=pltpu.CompilerParams(
            vmem_limit_bytes=128 * 1024 * 1024,
            disable_bounds_checks=True,
            disable_semaphore_checks=True,
            flags={"XLA_TPU_RESCHEDULE_DMA_DONES": True},
        ),
    )(xt, w, b)
    return jnp.transpose(out.reshape(B, 9, 8, 32, 8, 128), (0, 3, 5, 1, 2, 4)).reshape(B, S, F)
```

```python
import jax
import jax.numpy as jnp
from jax import lax
import jax.experimental.pallas as pl
import jax.experimental.pallas.tpu as pltpu

F32, BF16 = jnp.float32, jnp.bfloat16

STRASSEN = {
    1: ({(0, 0): 1, (1, 1): 1}, {(0, 0): 1, (1, 1): 1}),
    2: ({(1, 0): 1, (1, 1): 1}, {(0, 0): 1}),
    3: ({(0, 0): 1}, {(0, 1): 1, (1, 1): -1}),
    4: ({(1, 1): 1}, {(1, 0): 1, (0, 0): -1}),
    5: ({(0, 0): 1, (0, 1): 1}, {(1, 1): 1}),
    6: ({(1, 0): 1, (0, 0): -1}, {(0, 0): 1, (0, 1): 1}),
    7: ({(0, 1): 1, (1, 1): -1}, {(1, 0): 1, (1, 1): 1}),
}
RESULT = {(0, 0): {1: 1, 4: 1, 5: -1, 7: 1}, (0, 1): {3: 1, 5: 1},
          (1, 0): {2: 1, 4: 1}, (1, 1): {1: 1, 2: -1, 3: 1, 6: 1}}
NESTED = (2, 3, 4, 5)
ORDER = (None, (1, 4), (0, 2), (0, 1), None, (1, 2), (0, 4), (1, 1),
         (0, 5), (0, 7), (1, 5), (1, 7), (1, 3), (0, 3), (1, 6), (0, 6))
GROUP_WORK = 16 + 2 * (7 * 8 - len(NESTED))

RING = 9
DELAY = 58
W_FROM = 248
READ_ORDER = tuple(24 * i + -j % 24 for j in range(24) for i in range(6))


def _combine(terms):
    terms = list(terms)
    acc = terms.pop(next(k for k, (c, _) in enumerate(terms) if c > 0))[1]
    for c, v in terms:
        acc = acc + v if c > 0 else acc - v
    return acc


def _prune_packed(u):
    mate = lax.broadcasted_iota(jnp.int32, u.shape, 0) ^ 1
    lo = pltpu.bitcast((u << 16) & 0x7FFFFFFF, F32)
    hi = pltpu.bitcast(u & 0x7FFF0000, F32)
    big, small = jnp.maximum(lo, hi), jnp.minimum(lo, hi)
    nbig = jnp.take_along_axis(big, mate, axis=0, mode="promise_in_bounds")
    nsmall = jnp.take_along_axis(small, mate, axis=0, mode="promise_in_bounds")
    thr = jnp.maximum(jnp.minimum(big, nbig), jnp.maximum(small, nsmall))
    return u & (jnp.where(lo < thr, 0, 0xFFFF) | jnp.where(hi < thr, 0, -65536))


def _weight_forms():
    tall, short = {}, {}
    for g in range(2):
        tile = lambda k, s: 2 * k + s if 2 * k + s < 3 else 3 + g
        for m, (a, _) in STRASSEN.items():
            if m in NESTED:
                for n, (a2, _) in STRASSEN.items():
                    short[g, m, n] = tuple(sorted(
                        ((2 * i + i2, tile(k, s)), c * c2)
                        for (i, k), c in a.items() for (i2, s), c2 in a2.items()))
            else:
                for s in range(2):
                    tall[g, m, s] = tuple(sorted(((2 * i, tile(k, s)), c) for (i, k), c in a.items()))
    for q in range(4):
        short["E", q] = (((q, 5), 1),)
    return tall, short


def _distinct(forms):
    return list(dict.fromkeys(forms.values()))


def _prepare_weights(wbuf, tall_ref, short_ref):
    D, F = wbuf.shape
    u = pltpu.bitcast(wbuf[...], jnp.int32)
    rows = [_prune_packed(u[8 * i:8 * i + 8]) for i in range(D // 16)]
    rows = rows[:32] + rows[24:28] + rows[32:36] + rows[28:36]
    a = pltpu.bitcast(jnp.concatenate(rows, axis=0), BF16).T
    where = {}
    for forms, ref in zip(_weight_forms(), (tall_ref, short_ref)):
        block = lambda q, t: a[q * F // 4:q * F // 4 + 2 * ref.shape[1], t * 128:(t + 1) * 128]
        for slot, form in enumerate(_distinct(forms)):
            if len(form) == 1:
                v = block(*form[0][0])
            else:
                v = _combine((c, block(q, t).astype(F32)) for (q, t), c in form).astype(BF16)
            ref[slot] = pltpu.bitcast(v, jnp.int32)
        where.update({name: (ref, _distinct(forms).index(form)) for name, form in forms.items()})
    return lambda *name: pltpu.bitcast(where[name][0][where[name][1]], BF16)


def _group(load, weights, bias_ref, store, progress):
    Q = bias_ref.shape[0] // 4
    loaded, prods, shared, stored, arrival = {}, {}, {}, set(), []

    def x_blocks(k, n, pair, h):
        if (k, n, pair) not in loaded:
            loaded[k, n, pair] = load(k, n, pair).astype(F32).reshape(8 * n, 2, 8, 128)
        return loaded[k, n, pair][:, h].reshape(64 * n, 128)

    def x_tile(g, t, j, h):
        if t < 3:
            return x_blocks(2 * t, 2, 2 * g + j, h)
        diff = x_blocks(7 + g, 1, 2 * g + j, h) - x_blocks(7 + g, 1, 2 * (1 - g) + j, h)
        return jnp.concatenate([x_blocks(6, 1, 2 * g + j, h), diff], axis=0)

    def dot(a, b):
        return jnp.dot(a, b.astype(BF16), preferred_element_type=F32)

    e_todo = [(2 * i + q, j, h) for i, j in ((1, 0), (0, 0), (0, 1), (1, 1))
              for h in range(2) for q in range(2)]

    def shared_pass():
        q, j, h = e_todo.pop(0)
        rhs = jnp.concatenate([x_blocks(7, 1, 2 + j, h), x_blocks(8, 1, j, h)], axis=0)
        shared[q, j, h] = dot(weights("E", q), rhs) + bias_ref[pl.ds(q * Q, Q)]
        arrival.append(("E", q // 2, j))
        progress(1)

    def product(g, m):
        operand = lambda s, h: _combine(
            (c, x_tile(g, 2 * k + s, j, h)) for (k, j), c in STRASSEN[m][1].items())
        if m in NESTED:
            mm = lambda n: dot(weights(g, m, n), _combine(
                (c, operand(s, h)) for (s, h), c in STRASSEN[n][1].items()))
            n5, n1, n4, n7 = mm(5), mm(1), mm(4), mm(7)
            c11 = (n1 + n4) + (n7 - n5)
            progress(4)
            n2, n3, n6 = mm(2), mm(3), mm(6)
            shared_pass()
            progress(3)
            prods[g, m] = (jnp.concatenate([c11, n2 + n4], axis=0),
                           jnp.concatenate([n3 + n5, n6 + (n3 - n2) + n1], axis=0))
        else:
            p = [dot(weights(g, m, s), operand(s, h)) for h in range(2) for s in range(2)]
            prods[g, m] = (p[0] + p[1], p[2] + p[3])
            progress(8)
        arrival.append((g, m))

    def finish(g, i, j):
        values = []
        for h in range(2):
            terms = {(g, m): (c, prods[g, m][h]) for m, c in RESULT[i, j].items()}
            terms["E", i, j] = (1, jnp.concatenate([shared[2 * i + q, j, h] for q in range(2)], axis=0))
            values.append(_combine(terms[k] for k in sorted(terms, key=arrival[::-1].index)))
        nested = arrival[-1][1] in NESTED
        store(i, 2 * g + j, values, sorted(range(Q // 4), key=lambda k: k % (Q // 8) if nested else k))

    for step in ORDER:
        if step is None:
            for _ in range(4):
                shared_pass()
        else:
            product(*step)
        loaded.clear()
        for g in range(2):
            for (i, j), ms in RESULT.items():
                if ((g, i, j) not in stored and all((g, m) in prods for m in ms)
                        and (2 * i + 1, j, 1) in shared):
                    finish(g, i, j)
                    stored.add((g, i, j))
    assert len(stored) == 8


def _kernel(x_hbm, w_hbm, b_hbm, o_hbm, xbuf, obuf, wbuf, bbuf, tall_ref, short_ref, bias_ref,
            xsem, first_sem, osem):
    F = w_hbm.shape[1]
    B = x_hbm.shape[0]
    wrap = lambda s: jnp.where(s >= RING, s - RING, s)

    def read(b, slot, at, sem, priority):
        pltpu.make_async_copy(x_hbm.at[(b, *at)], xbuf.at[(slot, *at)], sem).start(priority=priority)

    def finish(part, sem):
        pltpu.make_async_copy(part, part, sem).wait()

    def blocks_of(ref, p, e):
        return ref.at[p, pl.ds(4 * e, 5), e], ref.at[p, pl.ds(5 * e, 4), 1 - e]

    def write(src, dst, half):
        for q in range(2):
            cols = pl.ds(8 * half + 4 * q, 4)
            pltpu.make_async_copy(src.at[:, cols], dst.at[:, cols], osem.at[0]).start()

    def write_pair(p, n):
        write(*(ref.at[p, :, n >> 4, (n >> 1) & 7] for ref in (obuf, o_hbm)), n & 1)

    def write_last(e, odd, r, half):
        write(*(blocks_of(ref, B // 2 - 1, e)[odd].at[:, r] for ref in (obuf, o_hbm)), half)

    params = [pltpu.make_async_copy(b_hbm, bbuf, first_sem.at[3]),
              pltpu.make_async_copy(w_hbm, wbuf, first_sem.at[4])]
    for copy in params:
        copy.start()
    for u in range(2):
        for r in range(8):
            read(0, 0, (slice(None), r, pl.ds(4 * u, 4)), first_sem.at[u], 1)
    for copy in params:
        copy.wait()
    weights = _prepare_weights(wbuf, tall_ref, short_ref)
    bias_ref[...] = jnp.broadcast_to(bbuf[...].reshape(1, F).astype(F32), (128, F)).T

    def batch(t, _):
        slot = wrap(t)
        pl.when(t > 0)(lambda: finish(xbuf.at[slot], xsem.at[slot]))
        slots = [wrap(2 * t + e) for e in range(3)]
        blocks = blocks_of(obuf, t >> 1, t & 1)
        work = 0

        def progress(n):
            nonlocal work
            span, work = (work, work + n), work + n
            per = len(READ_ORDER)
            due = range(*(per - DELAY + v * per // (2 * GROUP_WORK) for v in span))
            for e in range(3):
                ks = [k % per for k in due if k // per == e]
                if ks:
                    @pl.when(jnp.logical_and(2 * t + e > 0, 2 * t + e < B))
                    def _():
                        for k in ks:
                            g = READ_ORDER[k]
                            at = (g >> 4, (g >> 1) & 7, pl.ds(8 * (g & 1), 8))
                            read(2 * t + e, slots[e], at, xsem.at[slots[e]], k % 2)
            ks = range(*(min(72, v * 72 * per // (2 * GROUP_WORK * DELAY)) for v in span))
            if ks:
                @pl.when(t == 0)
                def _():
                    for k in ks:
                        read(0, 0, (k % 9, k // 9, pl.ds(8, 8)), first_sem.at[2], k % 2)
            for k in range(*(pl.cdiv(v * 8, GROUP_WORK) for v in span)):
                dp, n = divmod(k - W_FROM, 32)
                pl.when(jnp.logical_and(t + dp >= 0, t + dp < B // 2 - 2))(lambda: write_pair(t + dp, n))
                pl.when(t == B - 2)(lambda: write_pair(B // 2 - 2, k))
                if k < 25 and k != 16:
                    @pl.when(t == B - 1)
                    def _():
                        for q in range(2):
                            if k < 16:
                                write_last(0, *divmod(k, 8), q)
                            else:
                                write_last(1, *divmod(2 * (k - 17) + q, 8), 0)

        for u in range(4):
            def load(k, n, pair):
                return xbuf[slot, pl.ds(k, n), :, 4 * u + pair]

            def store(i, pair, values, rows):
                v = jnp.concatenate([a.reshape(36, 8, 128) for a in values], axis=1).astype(obuf.dtype)
                for k in rows:
                    block, r = divmod(36 * i + k, 8)
                    blocks[block % 2][block // 2, r, 4 * u + pair] = v[k]

            if u < 3:
                part = xbuf.at[0, :, :, pl.ds(4 * u, 8 if u == 2 else 4)]
                pl.when(t == 0)(lambda: finish(part, first_sem.at[u]))
            _group(load, weights, bias_ref, store, progress)

    assert W_FROM >= 32 * (B // 2 - 1)
    lax.fori_loop(0, B, batch, None)
    for k in range(16):
        write_last(1, *divmod(k, 8), 1)
    finish(obuf, osem.at[0])


@jax.jit
def pallas_standalone__structured_sparse_n_m__ragged_kernel(
    x: jax.Array,
    w: jax.Array,
    b: jax.Array,
):
    B, S, D = x.shape
    F = w.shape[1]
    assert (B, S, D, F) == (16, 4096, 576, 576)
    tall, short = _weight_forms()
    xt = jnp.transpose(x.reshape(B, 32, 128, 9, 8, 8), (0, 3, 4, 1, 5, 2)).reshape(B, 9, 8, 16, 16, 128)
    out_shape = (B // 2, 9, 2, *xt.shape[2:])
    out = pl.pallas_call(
        _kernel,
        in_specs=[pl.BlockSpec(memory_space=pl.ANY)] * 3,
        out_specs=pl.BlockSpec(memory_space=pl.ANY),
        out_shape=jax.ShapeDtypeStruct(out_shape, x.dtype),
        scratch_shapes=[
            pltpu.VMEM((RING, *xt.shape[1:]), x.dtype),
            pltpu.VMEM(out_shape, x.dtype),
            pltpu.VMEM((D, F), w.dtype),
            pltpu.VMEM((F,), b.dtype),
            pltpu.VMEM((len(_distinct(tall)), F // 4, 128), jnp.int32),
            pltpu.VMEM((len(_distinct(short)), F // 8, 128), jnp.int32),
            pltpu.VMEM((F, 128), F32),
            pltpu.SemaphoreType.DMA((RING,)),
            pltpu.SemaphoreType.DMA((5,)),
            pltpu.SemaphoreType.DMA((1,)),
        ],
        compiler_params=pltpu.CompilerParams(
            vmem_limit_bytes=128 * 1024 * 1024,
            disable_bounds_checks=True,
            disable_semaphore_checks=True,
            flags={"XLA_TPU_RESCHEDULE_DMA_DONES": True},
        ),
    )(xt, w, b)
    return jnp.transpose(out.reshape(B, 9, 8, 32, 8, 128), (0, 3, 5, 1, 2, 4)).reshape(B, S, F)
```
